```python
import jax
import jax.numpy as jnp

def _softmax(x, axis=-1):
    return jax.nn.softmax(x, axis=axis)

def _gelu(x):
    return jax.nn.gelu(x, approximate=True)

def _silu(x):
    return jax.nn.silu(x)

def _sigmoid(x):
    return jax.nn.sigmoid(x)

def _layernorm(x, axis=-1, eps=1e-05):
    m = jnp.mean(x, axis=axis, keepdims=True)
    v = jnp.var(x, axis=axis, keepdims=True)
    return (x - m) / jnp.sqrt(v + eps)

def _scatter_add(tgt, idx, src, axis=0):
    return tgt.at[idx].add(src)

def _segment_sum(src, seg, n):
    return jax.ops.segment_sum(src, seg, n)

class _Rng:

    def __init__(self, key):
        self._k = key

    def _next(self):
        self._k, sub = jax.random.split(self._k)
        return sub

    def normal(self, shape):
        return jax.random.normal(self._next(), shape, dtype=jnp.bfloat16)

    def randint(self, lo, hi, shape):
        return jax.random.randint(self._next(), shape, lo, hi, dtype=jnp.int32)

    def uniform(self, shape, lo=0.0, hi=1.0):
        return jax.random.uniform(self._next(), shape, jnp.bfloat16, lo, hi)

    def permutation(self, n):
        return jax.random.permutation(self._next(), n)
kernel_name = 'interleave_layers__memory_aug_recurrent_mem_tr__glu_gated_geglu__prompt'

def setup_inputs():
    _rng = _Rng(jax.random.key(int.from_bytes(__import__("os").urandom(4), "little")))
    _w = lambda a: (lambda t: t.astype(jnp.bfloat16) if jnp.issubdtype(t.dtype, jnp.floating) else t)(jnp.asarray(a))

    def _A_setup():
        B, S, Dm = (1, 2048, 1024)
        H, Dh = (32, 128)
        M, seg = (8, 32)
        seg = min(seg, S)
        S = S // seg * seg
        return {'x': _w((lambda *s: _rng.normal(s) * 0.05)(B, S, Dm)), 'mem0': _w((lambda *s: _rng.normal(s) * 0.05)(B, M, Dm)), 'Wq': _w((lambda *s: _rng.normal(s) * 0.05)(Dm, H, Dh) * Dm ** (-0.5)), 'Wk': _w((lambda *s: _rng.normal(s) * 0.05)(Dm, H, Dh) * Dm ** (-0.5)), 'Wv': _w((lambda *s: _rng.normal(s) * 0.05)(Dm, H, Dh) * Dm ** (-0.5)), 'Wo': _w((lambda *s: _rng.normal(s) * 0.05)(H, Dh, Dm) * (H * Dh) ** (-0.5)), 'seg_len': seg}
    _A_in = _A_setup()

    def _B_setup():
        B, S, Dm, Df = (1, 2048, 1024, 3584)
        return {'x': _w((lambda *s: _rng.normal(s) * 0.05)(B, S, Dm)), 'w_gate': _w((lambda *s: _rng.normal(s) * 0.05)(Dm, Df) * Dm ** (-0.5)), 'w_up': _w((lambda *s: _rng.normal(s) * 0.05)(Dm, Df) * Dm ** (-0.5)), 'w_down': _w((lambda *s: _rng.normal(s) * 0.05)(Df, Dm) * Df ** (-0.5))}
    _B_in = _B_setup()
    return {'A_x': _A_in['x'], 'A_mem0': _A_in['mem0'], 'A_Wq': _A_in['Wq'], 'A_Wk': _A_in['Wk'], 'A_Wv': _A_in['Wv'], 'A_Wo': _A_in['Wo'], 'A_seg_len': _A_in['seg_len'], 'B_x': _B_in['x'], 'B_w_gate': _B_in['w_gate'], 'B_w_up': _B_in['w_up'], 'B_w_down': _B_in['w_down']}

def reference(A_x, A_mem0, A_Wq, A_Wk, A_Wv, A_Wo, A_seg_len, B_x, B_w_gate, B_w_up, B_w_down):

    def _A_ref(x, mem0, Wq, Wk, Wv, Wo, seg_len):
        B, S, Dm = x.shape
        H, Dh = (Wq.shape[1], Wq.shape[2])
        M = mem0.shape[1]
        scale = Dh ** (-0.5)
        n_seg = S // seg_len
        L = M + seg_len
        idx = jnp.arange(L)
        mask = (idx[:, None] < M) | (idx[:, None] >= idx[None, :])
        mem = mem0
        outs = []
        for s in range(n_seg):
            xs = x[:, s * seg_len:(s + 1) * seg_len, :].copy()
            h = jnp.concatenate([mem, xs], axis=1)
            q = jnp.einsum('btd,dhe->bhte', h, Wq)
            k = jnp.einsum('btd,dhe->bhte', h, Wk)
            v = jnp.einsum('btd,dhe->bhte', h, Wv)
            scores = jnp.einsum('bhqe,bhke->bhqk', q, k) * scale
            scores = jnp.where(mask[None, None], scores, -1000000000.0)
            p = _softmax(scores, axis=-1)
            o = jnp.einsum('bhqk,bhke->bhqe', p, v)
            o = jnp.einsum('bhte,hed->btd', o, Wo)
            mem = o[:, :M, :].copy()
            outs.append(o[:, M:, :])
        return jnp.concatenate(outs, axis=1)

    def _B_ref(x, w_gate, w_up, w_down):
        g = jnp.einsum('bsd,df->bsf', x, w_gate)
        u = jnp.einsum('bsd,df->bsf', x, w_up)
        h = _gelu(g) * u
        return jnp.einsum('bsf,fd->bsd', h, w_down)
    x = A_x
    x = x + _A_ref(_layernorm(x, axis=-1), A_mem0, A_Wq, A_Wk, A_Wv, A_Wo, A_seg_len)
    x = x + _B_ref(_layernorm(x, axis=-1), B_w_gate, B_w_up, B_w_down)
    x = x + _A_ref(_layernorm(x, axis=-1), A_mem0, A_Wq, A_Wk, A_Wv, A_Wo, A_seg_len)
    x = x + _B_ref(_layernorm(x, axis=-1), B_w_gate, B_w_up, B_w_down)
    return x
```

```python
import functools

import jax
import jax.numpy as jnp
import numpy as np
from jax import lax
import jax.experimental.pallas as pl
import jax.experimental.pallas.tpu as pltpu

F32 = jnp.float32
BF16 = jnp.bfloat16
LANES = 128
LAG = 4
HEAD_GROUP = 4
FF_CHUNK = 512
OUT_CHUNK = 512
EPS = 1e-5


def _layernorm(x):
    m = jnp.mean(x, axis=-1, keepdims=True)
    c = x - m
    v = jnp.mean(c * c, axis=-1, keepdims=True)
    return c * lax.rsqrt(v + EPS)


def _gelu(x):
    c = float(np.sqrt(2.0 / np.pi))
    return x * (0.5 * (1.0 + jnp.tanh(c * (x + 0.044715 * (x * x * x)))))


def _dot(a, b):
    return jnp.dot(a, b, preferred_element_type=F32)


def _dot_nt(a, b):
    return lax.dot_general(a, b, (((1,), (1,)), ((), ())), preferred_element_type=F32)


def _score_mask(n_layers, n_mem, seg):
    rows = n_layers * (n_mem + seg)

    def layer_and_pos(i):
        layer = jnp.zeros_like(i)
        pos = i
        for l in range(1, n_layers):
            in_mem = (i >= l * n_mem) & (i < (l + 1) * n_mem)
            layer = jnp.where(in_mem, l, layer)
            pos = jnp.where(in_mem, i - l * n_mem, pos)
        for l in range(n_layers):
            lo = n_layers * n_mem + l * seg
            in_seg = (i >= lo) & (i < lo + seg)
            layer = jnp.where(in_seg, l, layer)
            pos = jnp.where(in_seg, i - lo + n_mem, pos)
        return layer, pos

    r_layer, r_pos = layer_and_pos(lax.broadcasted_iota(jnp.int32, (rows, rows), 0))
    c_layer, c_pos = layer_and_pos(lax.broadcasted_iota(jnp.int32, (rows, rows), 1))
    same = r_layer == c_layer
    keep = same & ((r_pos < n_mem) | (r_pos >= c_pos))
    fill = jnp.where(same, -1e9, -jnp.inf).astype(F32)
    return keep, fill


def _kernel(x_hbm, mem0_ref, wq_hbm, wk_hbm, wv_hbm, wo_hbm, wg_hbm, wu_hbm, wd_hbm,
            out_hbm,
            wq, wk, wv, wo, wg, wu, wd, stage, xin, xs, xout, h2, h1, att, hf, act,
            stage_sem, w_sem, x_sem, out_sem, *, n_heads, n_mem, seg, n_seg):
    dm = wq.shape[0]
    dh = LANES
    dff = wg.shape[1]
    scale = float(dh) ** -0.5
    n_groups = n_heads // HEAD_GROUP
    gw = HEAD_GROUP * dh

    def rows(s):
        return pl.ds(pl.multiple_of(s * seg, seg), seg)

    def attend(h_ref, n_layers, fillers=()):
        n = n_layers * (n_mem + seg)
        n_pad = h_ref.shape[0]
        keep, fill = _score_mask(n_layers, n_mem, seg)
        if n_pad != n:
            keep, fill = _pad_mask(keep, fill, n_pad)
        fillers = list(fillers)

        def project(g):
            h = h_ref[...]
            cols = slice(g * gw, (g + 1) * gw)
            return tuple(_dot(h, w[:, cols]).astype(BF16) for w in (wq, wk, wv))

        def scores(q, k):
            out = []
            for i in range(HEAD_GROUP):
                c = slice(i * dh, (i + 1) * dh)
                s = jnp.where(keep, _dot_nt(q[:, c], k[:, c]) * scale, fill)
                e = jnp.exp(s - jnp.max(s, axis=-1, keepdims=True))
                out.append((e.astype(BF16), 1.0 / jnp.sum(e, axis=-1, keepdims=True)))
            return out

        def mix(g, probs, v):
            for i, (e, inv) in enumerate(probs):
                o = _dot(e, v[:, i * dh:(i + 1) * dh]) * inv
                c = g * gw + i * dh
                att[0:n_pad, c:c + dh] = o.astype(BF16)

        qkv = project(0)
        pending = None
        for g in range(n_groups):
            probs = scores(qkv[0], qkv[1])
            v = qkv[2]
            if pending is not None:
                mix(*pending)
            pending = (g, probs, v)
            if g + 1 < n_groups:
                qkv = project(g + 1)
            elif fillers:
                fillers.pop(0)()
        mix(*pending)
        for f in fillers:
            f()

    def out_project(h_ref, n_layers, segs):
        n_pad = h_ref.shape[0]
        a = att[0:n_pad, :]
        for j in range(dm // OUT_CHUNK):
            cols = slice(j * OUT_CHUNK, (j + 1) * OUT_CHUNK)
            o = _dot(a, wo[:, cols])
            if n_layers == 2:
                h_ref[0:2 * n_mem, cols] = o[0:2 * n_mem].astype(BF16)
            else:
                h_ref[0:n_pad, cols] = o.astype(BF16)
            for l, s in enumerate(segs):
                lo = n_layers * n_mem + l * seg
                from_input = n_layers == 2 and l == 0
                x = xin[rows(s), cols].astype(F32) if from_input else xs[rows(s), cols]
                xs[rows(s), cols] = x + o[lo:lo + seg]

    def ffn_norm(segs):
        for l, s in enumerate(segs):
            hf[l * seg:(l + 1) * seg, :] = _layernorm(xs[rows(s), :]).astype(BF16)

    def ffn_up(j):
        cols = slice(j * FF_CHUNK, (j + 1) * FF_CHUNK)
        h = hf[...]
        act[:, cols] = (_gelu(_dot(h, wg[:, cols])) * _dot(h, wu[:, cols])).astype(BF16)

    def ffn_down(segs):
        a = act[...]
        for j in range(dm // OUT_CHUNK):
            cols = slice(j * OUT_CHUNK, (j + 1) * OUT_CHUNK)
            o = _dot(a, wd[:, cols])
            for l, s in enumerate(segs):
                y = xs[rows(s), cols] + o[l * seg:(l + 1) * seg]
                xs[rows(s), cols] = y
                xout[rows(s), cols] = y.astype(BF16)

    def load_input(s):
        x = xin[rows(s), :].astype(F32)
        xs[rows(s), :] = x
        return _layernorm(x)

    k_chunks = dm // LANES
    chunk_rows = LANES * n_heads
    qkv = ((wq_hbm, wq), (wk_hbm, wk), (wv_hbm, wv))

    def stage_copy(src, c, slot):
        return pltpu.make_async_copy(
            src.at[pl.ds(pl.multiple_of(c * chunk_rows, chunk_rows), chunk_rows), :],
            stage.at[slot], stage_sem.at[slot])

    head_rows = (LAG + 1) * seg
    x_head = pltpu.make_async_copy(
        x_hbm.at[0:head_rows, :], xin.at[0:head_rows, :], x_sem.at[0])
    x_tail = pltpu.make_async_copy(
        x_hbm.at[head_rows:, :], xin.at[head_rows:, :], x_sem.at[1])
    wo_copy = pltpu.make_async_copy(wo_hbm, wo, w_sem.at[0])
    ff_copies = [pltpu.make_async_copy(s, d, w_sem.at[1 + i])
                 for i, (s, d) in enumerate(((wg_hbm, wg), (wu_hbm, wu), (wd_hbm, wd)))]

    x_head.start()
    for c in range(k_chunks):
        stage_copy(wq_hbm, c, c).start()

    pairs = n_heads // 2
    for i, (src, dst) in enumerate(qkv):
        def retile(c, carry, i=i, src=src, dst=dst):
            stage_copy(src, c, c).wait()
            words = stage.bitcast(jnp.uint32)
            d_rows = pl.ds(pl.multiple_of(c * LANES, LANES), LANES)
            for j in range(pairs):
                a = words[c, pl.ds(j, LANES // 2, stride=2 * pairs), :]
                b = words[c, pl.ds(j + pairs, LANES // 2, stride=2 * pairs), :]
                lo = (a & jnp.uint32(0xFFFF)) | (b << 16)
                hi = (a >> 16) | (b & jnp.uint32(0xFFFF0000))
                dst[d_rows, 2 * j * dh:(2 * j + 1) * dh] = pltpu.bitcast(lo, BF16)
                dst[d_rows, (2 * j + 1) * dh:(2 * j + 2) * dh] = pltpu.bitcast(hi, BF16)
            if i + 1 < len(qkv):
                stage_copy(qkv[i + 1][0], c, c).start()
            return carry

        lax.fori_loop(0, k_chunks, retile, 0)
        if i == 1:
            wo_copy.start()
    for cp in ff_copies:
        cp.start()
    x_tail.start()

    x_head.wait()
    mem0 = mem0_ref[...].astype(F32)
    pad1 = h1.shape[0] - n_mem - seg

    def set_single(mem, s_norm):
        h1[...] = jnp.concatenate(
            [mem, s_norm, jnp.zeros((pad1, dm), F32)], axis=0).astype(BF16)

    n_full = n_seg - LAG

    def step(it, carry):
        is_full = (it >= LAG) & (it < LAG + n_full)
        head = it < LAG
        tail = it >= LAG + n_full

        @pl.when(it == 0)
        def _():
            set_single(mem0, load_input(0))

        @pl.when(jnp.logical_not(is_full))
        def _():
            attend(h1, 1)

            @pl.when(it == 0)
            def _():
                wo_copy.wait()

            s = jnp.where(head, it, it - LAG)
            out_project(h1, 1, (s,))

            @pl.when(it < LAG - 1)
            def _():
                set_single(h1[0:2 * n_mem, :].astype(F32)[0:n_mem], load_input(it + 1))

            do_ffn = (it == LAG - 1) | (tail & ((it - LAG - n_full) != 2))

            @pl.when(do_ffn)
            def _():
                @pl.when(it == LAG - 1)
                def _():
                    for cp in ff_copies:
                        cp.wait()

                k = it - LAG - n_full
                first = jnp.where(head, 0, jnp.where(k == 0, n_seg - 1, n_full + k - 1))
                second = jnp.where(head, 1, jnp.where(k == 0, n_full - 1, n_full + k))
                segs = (first, second)
                ffn_norm(segs)
                for j in range(dff // FF_CHUNK):
                    ffn_up(j)
                ffn_down(segs)

            @pl.when(it == LAG - 1)
            def _():
                x_tail.wait()
                mem1 = h1[0:2 * n_mem, :].astype(F32)[0:n_mem]
                h2[0:2 * n_mem, :] = jnp.concatenate([mem1, mem0], axis=0).astype(BF16)
                h2[2 * n_mem:2 * n_mem + seg, :] = load_input(it + 1).astype(BF16)
                h2[2 * n_mem + seg:, :] = _layernorm(xs[rows(0), :]).astype(BF16)

            @pl.when(tail & (it < n_seg + LAG - 1))
            def _():
                set_single(h1[0:2 * n_mem, :].astype(F32)[0:n_mem],
                           _layernorm(xs[rows(it + 1 - LAG), :]))

        @pl.when(is_full)
        def _():
            t = it
            ff_segs = (t - 1, jnp.where(t == LAG, LAG - 2, t - LAG - 1))
            ffn_norm(ff_segs)
            attend(h2, 2, [functools.partial(ffn_up, j) for j in range(dff // FF_CHUNK)])
            out_project(h2, 2, (t, t - LAG))
            nxt = jnp.minimum(t + 1, n_seg - 1)
            xn = xin[rows(nxt), :].astype(F32)
            h2[2 * n_mem:2 * n_mem + seg, :] = _layernorm(xn).astype(BF16)
            h2[2 * n_mem + seg:, :] = _layernorm(xs[rows(t + 1 - LAG), :]).astype(BF16)
            ffn_down(ff_segs)

            @pl.when(t + 1 == n_seg)
            def _():
                mem2 = h2[0:2 * n_mem, :].astype(F32)[n_mem:]
                set_single(mem2, h2[2 * n_mem + seg:, :].astype(F32))
                done = (n_full - 1) * seg
                pltpu.make_async_copy(
                    xout.at[0:done, :], out_hbm.at[0:done, :], out_sem.at[0]).start()

        return carry

    lax.fori_loop(0, n_seg + LAG, step, 0)

    done = (n_full - 1) * seg
    last = pltpu.make_async_copy(xout.at[done:, :], out_hbm.at[done:, :], out_sem.at[1])
    last.start()
    pltpu.make_async_copy(xout.at[0:done, :], out_hbm.at[0:done, :], out_sem.at[0]).wait()
    last.wait()


def _pad_mask(keep, fill, n_pad):
    n = keep.shape[0]
    r = lax.broadcasted_iota(jnp.int32, (n_pad, n_pad), 0)
    c = lax.broadcasted_iota(jnp.int32, (n_pad, n_pad), 1)
    n_mem = 8
    keep = ((c < n) & ((r < n_mem) | (r >= c)))
    fill = jnp.where(c < n, -1e9, -jnp.inf).astype(F32)
    return keep, fill


@functools.partial(jax.jit, static_argnames=("A_seg_len",))
def pallas_interleave_layers__memory_aug_recurrent_mem_tr__glu_gated_geglu__prompt_kernel(
    A_x: jax.Array,
    A_mem0: jax.Array,
    A_Wq: jax.Array,
    A_Wk: jax.Array,
    A_Wv: jax.Array,
    A_Wo: jax.Array,
    A_seg_len: int,
    B_x: jax.Array,
    B_w_gate: jax.Array,
    B_w_up: jax.Array,
    B_w_down: jax.Array,
):
    del B_x
    b, s, dm = A_x.shape
    _, n_heads, dh = A_Wq.shape
    n_mem = A_mem0.shape[1]
    dff = B_w_gate.shape[1]
    seg = int(A_seg_len)
    n_seg = s // seg
    assert b == 1 and dh == LANES and n_seg * seg == s and n_mem == 8 and seg % 16 == 0
    assert LAG == 4 and n_seg > 2 * LAG
    hd = n_heads * dh
    full = 2 * (n_mem + seg)
    single = pl.cdiv(n_mem + seg, 16) * 16

    any_spec = pl.BlockSpec(memory_space=pl.ANY)
    out = pl.pallas_call(
        functools.partial(_kernel, n_heads=n_heads, n_mem=n_mem, seg=seg, n_seg=n_seg),
        out_shape=jax.ShapeDtypeStruct((s, dm), A_x.dtype),
        in_specs=[any_spec, pl.BlockSpec(memory_space=pltpu.VMEM)] + [any_spec] * 7,
        out_specs=any_spec,
        scratch_shapes=[
            pltpu.VMEM((dm, hd), BF16), pltpu.VMEM((dm, hd), BF16), pltpu.VMEM((dm, hd), BF16),
            pltpu.VMEM((hd, dm), BF16),
            pltpu.VMEM((dm, dff), BF16), pltpu.VMEM((dm, dff), BF16), pltpu.VMEM((dff, dm), BF16),
            pltpu.VMEM((dm // LANES, LANES * n_heads, dh), BF16),
            pltpu.VMEM((s, dm), BF16),
            pltpu.VMEM((s, dm), F32),
            pltpu.VMEM((s, dm), BF16),
            pltpu.VMEM((full, dm), BF16),
            pltpu.VMEM((single, dm), BF16),
            pltpu.VMEM((full, hd), BF16),
            pltpu.VMEM((2 * seg, dm), BF16),
            pltpu.VMEM((2 * seg, dff), BF16),
            pltpu.SemaphoreType.DMA((dm // LANES,)),
            pltpu.SemaphoreType.DMA((4,)),
            pltpu.SemaphoreType.DMA((2,)),
            pltpu.SemaphoreType.DMA((2,)),
        ],
        compiler_params=pltpu.CompilerParams(vmem_limit_bytes=110 * 1024 * 1024),
    )(
        A_x.reshape(s, dm),
        A_mem0.reshape(n_mem, dm),
        A_Wq.reshape(dm * n_heads, dh),
        A_Wk.reshape(dm * n_heads, dh),
        A_Wv.reshape(dm * n_heads, dh),
        A_Wo.reshape(hd, dm),
        B_w_gate,
        B_w_up,
        B_w_down,
    )
    return out.reshape(b, s, dm)
```

```python
import functools

import jax
import jax.numpy as jnp
import numpy as np
from jax import lax
import jax.experimental.pallas as pl
import jax.experimental.pallas.tpu as pltpu

F32 = jnp.float32
BF16 = jnp.bfloat16
LANES = 128
LAG = 4
HEAD_GROUP = 4
FF_TILES = 4
OUT_TILES = 4
EPS = 1e-5


def _layernorm(x):
    m = jnp.mean(x, axis=-1, keepdims=True)
    c = x - m
    v = jnp.mean(c * c, axis=-1, keepdims=True)
    return c * lax.rsqrt(v + EPS)


def _gelu(x):
    c = float(np.sqrt(2.0 / np.pi))
    return x * (0.5 * (1.0 + jnp.tanh(c * (x + 0.044715 * (x * x * x)))))


def _dot(a, b):
    return jnp.dot(a, b, preferred_element_type=F32)


def _dot_nt(a, b):
    return lax.dot_general(a, b, (((1,), (1,)), ((), ())), preferred_element_type=F32)


def _softmax(s):
    e = jnp.exp(s - jnp.max(s, axis=-1, keepdims=True))
    total = jnp.sum(e, axis=-1, keepdims=True)
    r = pl.reciprocal(total, approx=True)
    return e * (r * (2.0 - total * r))


def _score_mask(n_layers, n_mem, seg, n_pad):
    def layer_and_pos(i):
        layer = jnp.full_like(i, n_layers)
        pos = i
        for l in range(n_layers):
            in_mem = (i >= l * n_mem) & (i < (l + 1) * n_mem)
            lo = n_layers * n_mem + l * seg
            in_seg = (i >= lo) & (i < lo + seg)
            layer = jnp.where(in_mem | in_seg, l, layer)
            pos = jnp.where(in_mem, i - l * n_mem, jnp.where(in_seg, i - lo + n_mem, pos))
        return layer, pos

    r_layer, r_pos = layer_and_pos(lax.broadcasted_iota(jnp.int32, (n_pad, n_pad), 0))
    c_layer, c_pos = layer_and_pos(lax.broadcasted_iota(jnp.int32, (n_pad, n_pad), 1))
    same = r_layer == c_layer
    keep = same & ((r_pos < n_mem) | (r_pos >= c_pos))
    fill = jnp.where(same, -1e9, -jnp.inf).astype(F32)
    return keep, fill


def _load_tiles(ref, lo, n, rows=slice(None)):
    return jnp.concatenate([ref[t, rows, :] for t in range(lo, lo + n)], axis=1)


def _store_tiles(ref, lo, rows, val):
    for t in range(val.shape[1] // LANES):
        ref[lo + t, rows, :] = val[:, t * LANES:(t + 1) * LANES].astype(ref.dtype)


def _kernel(x_hbm, mem0_ref, wq_hbm, wk_hbm, wv_hbm, wo_hbm, wg_hbm, wu_hbm, wd_hbm,
            out_hbm,
            wq, wk, wv, wo, wg, wu, wd, stage, xin, xs, xout, h2, h1, att, hf, act,
            stage_sem, w_sem, x_sem, out_sem, *, n_mem, seg, n_seg):
    n_heads, dm, dh = wq.shape
    dm_tiles = dm // LANES
    ff_tiles = wg.shape[0]
    scale = float(dh) ** -0.5
    n_groups = n_heads // HEAD_GROUP
    every = slice(None)

    def rows(s):
        return pl.ds(pl.multiple_of(s * seg, seg), seg)

    def attend(h_ref, n_layers, fillers=()):
        n_pad = h_ref.shape[1]
        keep, fill = _score_mask(n_layers, n_mem, seg, n_pad)
        fillers = list(fillers)

        def project(g):
            h = _load_tiles(h_ref, 0, dm_tiles)
            out = []
            for w in (wq, wk, wv):
                y = _dot(h, _load_tiles(w, g * HEAD_GROUP, HEAD_GROUP))
                out.append([y[:, i * dh:(i + 1) * dh].astype(BF16) for i in range(HEAD_GROUP)])
            return out

        def mix(g, probs, v):
            for i in range(HEAD_GROUP):
                att[g * HEAD_GROUP + i, 0:n_pad, :] = _dot(probs[i], v[i]).astype(BF16)

        q, k, v = project(0)
        pending = None
        for g in range(n_groups):
            probs = [_softmax(jnp.where(keep, _dot_nt(q[i], k[i]) * scale, fill)).astype(BF16)
                     for i in range(HEAD_GROUP)]
            if pending is not None:
                mix(*pending)
            pending = (g, probs, v)
            if g + 1 < n_groups:
                q, k, v = project(g + 1)
            elif fillers:
                fillers.pop(0)()
        mix(*pending)
        for f in fillers:
            f()

    def out_project(h_ref, n_layers, segs):
        n_pad = h_ref.shape[1]
        a = _load_tiles(att, 0, n_heads, slice(0, n_pad))
        for j in range(0, dm_tiles, OUT_TILES):
            cols = slice(j * LANES, (j + OUT_TILES) * LANES)
            o = _dot(a, _load_tiles(wo, j, OUT_TILES))
            _store_tiles(h_ref, j, slice(0, 2 * n_mem), o[0:2 * n_mem])
            for l, s in enumerate(segs):
                lo = n_layers * n_mem + l * seg
                from_input = n_layers == 2 and l == 0
                x = xin[rows(s), cols].astype(F32) if from_input else xs[rows(s), cols]
                xs[rows(s), cols] = x + o[lo:lo + seg]

    def ffn_norm(segs):
        for l, s in enumerate(segs):
            _store_tiles(hf, 0, slice(l * seg, (l + 1) * seg), _layernorm(xs[rows(s), :]))

    def ffn_up(j):
        h = _load_tiles(hf, 0, dm_tiles)
        g = _dot(h, _load_tiles(wg, j, FF_TILES))
        u = _dot(h, _load_tiles(wu, j, FF_TILES))
        _store_tiles(act, j, every, _gelu(g) * u)

    def ffn_down(segs):
        a = _load_tiles(act, 0, ff_tiles)
        for j in range(0, dm_tiles, OUT_TILES):
            cols = slice(j * LANES, (j + OUT_TILES) * LANES)
            o = _dot(a, _load_tiles(wd, j, OUT_TILES))
            for l, s in enumerate(segs):
                y = xs[rows(s), cols] + o[l * seg:(l + 1) * seg]
                xs[rows(s), cols] = y
                xout[rows(s), cols] = y.astype(BF16)

    def load_input(s):
        x = xin[rows(s), :].astype(F32)
        xs[rows(s), :] = x
        return _layernorm(x)

    chunk_rows = LANES * n_heads
    qkv = ((wq_hbm, wq), (wk_hbm, wk), (wv_hbm, wv))

    def stage_copy(src, c):
        return pltpu.make_async_copy(
            src.at[pl.ds(pl.multiple_of(c * chunk_rows, chunk_rows), chunk_rows), :],
            stage.at[c], stage_sem.at[c])

    def tile_copies(src, dst, sem):
        return [pltpu.make_async_copy(src.at[:, t * LANES:(t + 1) * LANES], dst.at[t], sem)
                for t in range(dst.shape[0])]

    head_rows = (LAG + 1) * seg
    x_head = pltpu.make_async_copy(
        x_hbm.at[0:head_rows, :], xin.at[0:head_rows, :], x_sem.at[0])
    x_tail = pltpu.make_async_copy(
        x_hbm.at[head_rows:, :], xin.at[head_rows:, :], x_sem.at[1])
    wo_copies = tile_copies(wo_hbm, wo, w_sem.at[0])
    ff_copies = [cp for i, (src, dst) in enumerate(((wg_hbm, wg), (wu_hbm, wu), (wd_hbm, wd)))
                 for cp in tile_copies(src, dst, w_sem.at[1 + i])]

    x_head.start()
    for c in range(dm_tiles):
        stage_copy(wq_hbm, c).start()

    pairs = n_heads // 2
    for i, (src, dst) in enumerate(qkv):
        def retile(c, carry, i=i, src=src, dst=dst):
            stage_copy(src, c).wait()
            words = stage.bitcast(jnp.uint32)
            d_rows = pl.ds(pl.multiple_of(c * LANES, LANES), LANES)
            for j in range(pairs):
                a = words[c, pl.ds(j, LANES // 2, stride=2 * pairs), :]
                b = words[c, pl.ds(j + pairs, LANES // 2, stride=2 * pairs), :]
                lo = (a & jnp.uint32(0xFFFF)) | (b << 16)
                hi = (a >> 16) | (b & jnp.uint32(0xFFFF0000))
                dst[2 * j, d_rows, :] = pltpu.bitcast(lo, BF16)
                dst[2 * j + 1, d_rows, :] = pltpu.bitcast(hi, BF16)
            if i + 1 < len(qkv):
                stage_copy(qkv[i + 1][0], c).start()
            return carry

        lax.fori_loop(0, dm_tiles, retile, 0)
        if i == 1:
            for cp in wo_copies:
                cp.start()
    for cp in ff_copies:
        cp.start()
    x_tail.start()

    x_head.wait()
    mem0 = mem0_ref[...].astype(F32)
    pad1 = h1.shape[1] - n_mem - seg

    def get_mem(h_ref, lo):
        return _load_tiles(h_ref, 0, dm_tiles, slice(0, 2 * n_mem)).astype(F32)[lo:lo + n_mem]

    def set_single(mem, s_norm):
        _store_tiles(h1, 0, every, jnp.concatenate(
            [mem, s_norm, jnp.zeros((pad1, dm), F32)], axis=0))

    first_rows = slice(2 * n_mem, 2 * n_mem + seg)
    second_rows = slice(2 * n_mem + seg, 2 * n_mem + 2 * seg)
    ff_steps = range(0, ff_tiles, FF_TILES)
    n_full = n_seg - LAG

    def step(it, carry):
        is_full = (it >= LAG) & (it < LAG + n_full)
        head = it < LAG
        tail = it >= LAG + n_full

        @pl.when(it == 0)
        def _():
            set_single(mem0, load_input(0))

        @pl.when(jnp.logical_not(is_full))
        def _():
            attend(h1, 1)

            @pl.when(it == 0)
            def _():
                for cp in wo_copies:
                    cp.wait()

            s = jnp.where(head, it, it - LAG)
            out_project(h1, 1, (s,))

            @pl.when(it < LAG - 1)
            def _():
                set_single(get_mem(h1, 0), load_input(it + 1))

            do_ffn = (it == LAG - 1) | (tail & ((it - LAG - n_full) != 2))

            @pl.when(do_ffn)
            def _():
                @pl.when(it == LAG - 1)
                def _():
                    for cp in ff_copies:
                        cp.wait()

                k = it - LAG - n_full
                first = jnp.where(head, 0, jnp.where(k == 0, n_seg - 1, n_full + k - 1))
                second = jnp.where(head, 1, jnp.where(k == 0, n_full - 1, n_full + k))
                segs = (first, second)
                ffn_norm(segs)
                for j in ff_steps:
                    ffn_up(j)
                ffn_down(segs)

            @pl.when(it == LAG - 1)
            def _():
                x_tail.wait()
                _store_tiles(h2, 0, slice(0, 2 * n_mem),
                             jnp.concatenate([get_mem(h1, 0), mem0], axis=0))
                _store_tiles(h2, 0, first_rows, load_input(it + 1))
                _store_tiles(h2, 0, second_rows, _layernorm(xs[rows(0), :]))

            @pl.when(tail & (it < n_seg + LAG - 1))
            def _():
                set_single(get_mem(h1, 0), _layernorm(xs[rows(it + 1 - LAG), :]))

        @pl.when(is_full)
        def _():
            t = it
            ff_segs = (t - 1, jnp.where(t == LAG, LAG - 2, t - LAG - 1))
            ffn_norm(ff_segs)
            attend(h2, 2, [functools.partial(ffn_up, j) for j in ff_steps])
            out_project(h2, 2, (t, t - LAG))
            nxt = jnp.minimum(t + 1, n_seg - 1)
            _store_tiles(h2, 0, first_rows, _layernorm(xin[rows(nxt), :].astype(F32)))
            _store_tiles(h2, 0, second_rows, _layernorm(xs[rows(t + 1 - LAG), :]))
            ffn_down(ff_segs)

            @pl.when(t + 1 == n_seg)
            def _():
                second = _load_tiles(h2, 0, dm_tiles, second_rows).astype(F32)
                set_single(get_mem(h2, n_mem), second)
                done = (n_full - 1) * seg
                pltpu.make_async_copy(
                    xout.at[0:done, :], out_hbm.at[0:done, :], out_sem.at[0]).start()

        return carry

    lax.fori_loop(0, n_seg + LAG, step, 0)

    done = (n_full - 1) * seg
    last = pltpu.make_async_copy(xout.at[done:, :], out_hbm.at[done:, :], out_sem.at[1])
    last.start()
    pltpu.make_async_copy(xout.at[0:done, :], out_hbm.at[0:done, :], out_sem.at[0]).wait()
    last.wait()


@functools.partial(jax.jit, static_argnames=("A_seg_len",))
def pallas_interleave_layers__memory_aug_recurrent_mem_tr__glu_gated_geglu__prompt_kernel(
    A_x: jax.Array,
    A_mem0: jax.Array,
    A_Wq: jax.Array,
    A_Wk: jax.Array,
    A_Wv: jax.Array,
    A_Wo: jax.Array,
    A_seg_len: int,
    B_x: jax.Array,
    B_w_gate: jax.Array,
    B_w_up: jax.Array,
    B_w_down: jax.Array,
):
    del B_x
    b, s, dm = A_x.shape
    _, n_heads, dh = A_Wq.shape
    n_mem = A_mem0.shape[1]
    dff = B_w_gate.shape[1]
    seg = int(A_seg_len)
    n_seg = s // seg
    assert b == 1 and dh == LANES and n_seg * seg == s and n_mem == 8 and seg % 16 == 0
    assert LAG == 4 and n_seg > 2 * LAG
    hd = n_heads * dh
    full = 2 * (n_mem + seg)
    single = pl.cdiv(n_mem + seg, 16) * 16

    def tiled(n_rows, n_cols):
        return pltpu.VMEM((n_cols // LANES, n_rows, LANES), BF16)

    any_spec = pl.BlockSpec(memory_space=pl.ANY)
    out = pl.pallas_call(
        functools.partial(_kernel, n_mem=n_mem, seg=seg, n_seg=n_seg),
        out_shape=jax.ShapeDtypeStruct((s, dm), A_x.dtype),
        in_specs=[any_spec, pl.BlockSpec(memory_space=pltpu.VMEM)] + [any_spec] * 7,
        out_specs=any_spec,
        scratch_shapes=[
            tiled(dm, hd), tiled(dm, hd), tiled(dm, hd), tiled(hd, dm),
            tiled(dm, dff), tiled(dm, dff), tiled(dff, dm),
            pltpu.VMEM((dm // LANES, LANES * n_heads, dh), BF16),
            pltpu.VMEM((s, dm), BF16),
            pltpu.VMEM((s, dm), F32),
            pltpu.VMEM((s, dm), BF16),
            tiled(full, dm),
            tiled(single, dm),
            tiled(full, hd),
            tiled(2 * seg, dm),
            tiled(2 * seg, dff),
            pltpu.SemaphoreType.DMA((dm // LANES,)),
            pltpu.SemaphoreType.DMA((4,)),
            pltpu.SemaphoreType.DMA((2,)),
            pltpu.SemaphoreType.DMA((2,)),
        ],
        compiler_params=pltpu.CompilerParams(vmem_limit_bytes=110 * 1024 * 1024),
    )(
        A_x.reshape(s, dm),
        A_mem0.reshape(n_mem, dm),
        A_Wq.reshape(dm * n_heads, dh),
        A_Wk.reshape(dm * n_heads, dh),
        A_Wv.reshape(dm * n_heads, dh),
        A_Wo.reshape(hd, dm),
        B_w_gate,
        B_w_up,
        B_w_down,
    )
    return out.reshape(b, s, dm)
```

```python
import functools

import jax
import jax.numpy as jnp
import numpy as np
from jax import lax
import jax.experimental.pallas as pl
import jax.experimental.pallas.tpu as pltpu

F32 = jnp.float32
BF16 = jnp.bfloat16
LANES = 128
LAG = 4
AHEAD = 8
STREAM_CHUNKS = 2
HEAD_GROUP = 4
FF_TILES = 4
OUT_TILES = 4
EPS = 1e-5


def _layernorm(x):
    m = jnp.mean(x, axis=-1, keepdims=True)
    c = x - m
    v = jnp.mean(c * c, axis=-1, keepdims=True)
    return c * lax.rsqrt(v + EPS)


def _gelu(x):
    c = float(np.sqrt(2.0 / np.pi))
    return x * (0.5 * (1.0 + jnp.tanh(c * (x + 0.044715 * (x * x * x)))))


def _dot(a, b):
    return jnp.dot(a, b, preferred_element_type=F32)


def _dot_nt(a, b):
    return lax.dot_general(a, b, (((1,), (1,)), ((), ())), preferred_element_type=F32)


def _softmax(s):
    e = jnp.exp(s - jnp.max(s, axis=-1, keepdims=True))
    total = jnp.sum(e, axis=-1, keepdims=True)
    r = pl.reciprocal(total, approx=True)
    return e * (r * (2.0 - total * r))


def _score_mask(n_layers, n_mem, seg):
    n = n_layers * (n_mem + seg)

    def layer_and_pos(i):
        layer = jnp.zeros_like(i)
        pos = i
        for l in range(n_layers):
            in_mem = (i >= l * n_mem) & (i < (l + 1) * n_mem)
            lo = n_layers * n_mem + l * seg
            in_seg = (i >= lo) & (i < lo + seg)
            layer = jnp.where(in_mem | in_seg, l, layer)
            pos = jnp.where(in_mem, i - l * n_mem, jnp.where(in_seg, i - lo + n_mem, pos))
        return layer, pos

    r_layer, r_pos = layer_and_pos(lax.broadcasted_iota(jnp.int32, (n, n), 0))
    c_layer, c_pos = layer_and_pos(lax.broadcasted_iota(jnp.int32, (n, n), 1))
    same = r_layer == c_layer
    keep = same & ((r_pos < n_mem) | (r_pos >= c_pos))
    fill = jnp.where(same, -1e9, -jnp.inf).astype(F32)
    return keep, fill


def _load_tiles(ref, lo, n, rows=slice(None)):
    return jnp.concatenate([ref[t, rows, :] for t in range(lo, lo + n)], axis=1)


def _store_operand(ref, lo, rows, val):
    for t in range(val.shape[1] // LANES):
        tile = val[:, t * LANES:(t + 1) * LANES].astype(BF16)
        ref[lo + t, rows, :] = tile.astype(ref.dtype)


def _kernel(x_hbm, mem0_ref, wq_hbm, wk_hbm, wv_hbm, wo_hbm, wg_hbm, wu_hbm, wd_hbm,
            out_hbm,
            wqkv, wo, wg, wu, wd, stage, xin, xs, xout, ha, ahead, h2, att2, h1, att1, hf, act,
            stage_sem, w_sem, x_sem, out_sem, *, n_mem, seg, n_seg):
    n_heads, dm_tiles = wqkv.shape[0] // 3, wqkv.shape[1]
    dh = LANES
    ff_tiles = wg.shape[0]
    scale = float(dh) ** -0.5
    n_groups = n_heads // HEAD_GROUP
    every = slice(None)
    mem_rows = slice(0, 2 * n_mem)
    first_rows = slice(2 * n_mem, 2 * n_mem + seg)
    second_rows = slice(2 * n_mem + seg, 2 * n_mem + 2 * seg)
    first_ahead = n_seg - AHEAD

    def rows(s):
        if isinstance(s, int):
            return slice(s * seg, (s + 1) * seg)
        return pl.ds(pl.multiple_of(s * seg, seg), seg)

    def attend(h_ref, att, n_layers, ahead_seg=None, fillers=()):
        keep, fill = _score_mask(n_layers, n_mem, seg)
        fillers = list(fillers)

        def operand(x):
            return x.astype(BF16).astype(h_ref.dtype)

        def project(g):
            if ahead_seg is None:
                h = _load_tiles(h_ref, 0, dm_tiles)
            else:
                h = jnp.concatenate([_load_tiles(h_ref, 0, dm_tiles, mem_rows),
                                     _load_tiles(h_ref, 0, dm_tiles, second_rows)], axis=0)
            out = []
            for i in range(3):
                tile = i * n_heads + g * HEAD_GROUP
                w = [pltpu.bitcast(wqkv[tile + j].reshape(dm_tiles * LANES // 2, dh), BF16)
                     for j in range(HEAD_GROUP)]
                y = _dot(h, jnp.concatenate(w, axis=1))
                heads = [y[:, j * dh:(j + 1) * dh] for j in range(HEAD_GROUP)]
                if ahead_seg is not None:
                    heads = [jnp.concatenate([z[mem_rows], ahead[tile + j, rows(ahead_seg), :],
                                              z[2 * n_mem:]], axis=0)
                             for j, z in enumerate(heads)]
                out.append([operand(z) for z in heads])
            return out

        def mix(g, probs, v):
            for i in range(HEAD_GROUP):
                att[g * HEAD_GROUP + i] = operand(_dot(probs[i], v[i]))

        q, k, v = project(0)
        pending = None
        for g in range(n_groups):
            probs = [operand(_softmax(jnp.where(keep, _dot_nt(q[i], k[i]) * scale, fill)))
                     for i in range(HEAD_GROUP)]
            if pending is not None:
                mix(*pending)
            pending = (g, probs, v)
            if g + 1 < n_groups:
                q, k, v = project(g + 1)
            elif fillers:
                fillers.pop(0)()
        mix(*pending)
        for f in fillers:
            f()

    def out_project(h_ref, att, segs, first_from_input):
        n_rows = len(segs) * n_mem
        a = _load_tiles(att, 0, n_heads)
        for j in range(0, dm_tiles, OUT_TILES):
            cols = slice(j * LANES, (j + OUT_TILES) * LANES)
            o = _dot(a, _load_tiles(wo, j, OUT_TILES))
            _store_operand(h_ref, j, slice(0, n_rows), o[0:n_rows])
            for l, s in enumerate(segs):
                if first_from_input and l == 0:
                    x = xin[rows(s), cols].astype(F32)
                else:
                    x = xs[rows(s), cols]
                xs[rows(s), cols] = x + o[n_rows + l * seg:n_rows + (l + 1) * seg]

    def ffn_norm(segs):
        for l, s in enumerate(segs):
            _store_operand(hf, 0, slice(l * seg, (l + 1) * seg), _layernorm(xs[rows(s), :]))

    def ffn_up(j):
        h = _load_tiles(hf, 0, dm_tiles)
        g = _dot(h, _load_tiles(wg, j, FF_TILES))
        u = _dot(h, _load_tiles(wu, j, FF_TILES))
        _store_operand(act, j, every, _gelu(g) * u)

    def ffn_down(segs):
        a = _load_tiles(act, 0, ff_tiles)
        for j in range(0, dm_tiles, OUT_TILES):
            cols = slice(j * LANES, (j + OUT_TILES) * LANES)
            o = _dot(a, _load_tiles(wd, j, OUT_TILES))
            for l, s in enumerate(segs):
                y = xs[rows(s), cols] + o[l * seg:(l + 1) * seg]
                xs[rows(s), cols] = y
                xout[rows(s), cols] = y.astype(BF16)

    def load_input(s):
        x = xin[rows(s), :].astype(F32)
        xs[rows(s), :] = x
        return _layernorm(x)

    chunk_rows = LANES * n_heads

    def stage_copy(src, c):
        return pltpu.make_async_copy(
            src.at[pl.ds(pl.multiple_of(c * chunk_rows, chunk_rows), chunk_rows), :],
            stage.at[c], stage_sem.at[c])

    def tile_copies(src, dst, sem):
        return [pltpu.make_async_copy(src.at[:, t * LANES:(t + 1) * LANES], dst.at[t], sem)
                for t in range(dst.shape[0])]

    def row_copy(src, dst, lo, hi, sem):
        return pltpu.make_async_copy(
            src.at[lo * seg:hi * seg, :], dst.at[lo * seg:hi * seg, :], sem)

    x_ahead = row_copy(x_hbm, xin, first_ahead, n_seg, x_sem.at[0])
    x_head = row_copy(x_hbm, xin, 0, LAG + 1, x_sem.at[1])
    x_rest = row_copy(x_hbm, xin, LAG + 1, first_ahead, x_sem.at[2])
    wo_copies = tile_copies(wo_hbm, wo, w_sem.at[0])
    up_copies = tile_copies(wg_hbm, wg, w_sem.at[1]) + tile_copies(wu_hbm, wu, w_sem.at[2])
    down_copies = tile_copies(wd_hbm, wd, w_sem.at[3])
    n_full = n_seg - LAG
    out_early = row_copy(xout, out_hbm, 0, n_full - 1, out_sem.at[0])
    out_mid = row_copy(xout, out_hbm, n_full - 1, n_seg - 2, out_sem.at[1])
    out_last = row_copy(xout, out_hbm, n_seg - 2, n_seg, out_sem.at[2])

    x_ahead.start()
    for c in range(dm_tiles):
        stage_copy(wq_hbm, c).start()
    x_head.start()

    x_ahead.wait()
    for s in range(AHEAD):
        x = xin[(first_ahead + s) * seg:(first_ahead + s + 1) * seg, :].astype(F32)
        _store_operand(ha, 0, slice(s * seg, (s + 1) * seg), _layernorm(x))

    pairs = n_heads // 2

    def retile(which, cur_src, next_src, i):
        chunks = [i * STREAM_CHUNKS + j for j in range(STREAM_CHUNKS)]
        for c in chunks:
            stage_copy(cur_src, c).wait()
        words = stage.bitcast(jnp.uint32)
        h = jnp.concatenate([ha[c] for c in chunks], axis=1)
        for g in range(n_groups):
            columns = []
            for j in range(g * HEAD_GROUP // 2, (g + 1) * HEAD_GROUP // 2):
                packed = [words[c, pl.ds(j, LANES, stride=pairs), :] for c in chunks]
                for half in range(2):
                    tile = which * n_heads + 2 * j + half
                    w = [pltpu.bitcast((p >> (16 * half)).astype(jnp.uint16), BF16)
                         for p in packed]
                    for c, wc in zip(chunks, w):
                        wqkv[tile, c] = pltpu.bitcast(wc, jnp.uint32)
                    columns.append(jnp.concatenate(w, axis=0))
            y = _dot(h, jnp.concatenate(columns, axis=1))
            for j in range(HEAD_GROUP):
                tile = which * n_heads + g * HEAD_GROUP + j
                ahead[tile] = jnp.where(i == 0, 0.0, ahead[tile]) + y[:, j * dh:(j + 1) * dh]
        if next_src is not None:
            for c in chunks:
                stage_copy(next_src, c).start()
        else:
            @pl.when(i == 1)
            def _():
                for cp in up_copies:
                    cp.start()

    sources = (wq_hbm, wk_hbm, wv_hbm, None)
    for which in range(3):
        if which == 2:
            for cp in wo_copies:
                cp.start()
        body = functools.partial(retile, which, sources[which], sources[which + 1])
        lax.fori_loop(0, dm_tiles // STREAM_CHUNKS, lambda i, c: (body(i), c)[1], 0)
    for cp in down_copies:
        cp.start()
    x_rest.start()

    x_head.wait()
    mem0 = mem0_ref[...].astype(F32)

    def set_single_tokens(normed):
        _store_operand(h1, 0, slice(n_mem, n_mem + seg), normed)

    def ffn_only(segs, wait):
        if wait is not None:
            @pl.when(wait)
            def _():
                for cp in up_copies:
                    cp.wait()
        ffn_norm(segs)
        for j in ff_steps:
            ffn_up(j)
        if wait is not None:
            @pl.when(wait)
            def _():
                for cp in down_copies:
                    cp.wait()
        ffn_down(segs)

    def single_step(it, head):
        attend(h1, att1, 1)
        if head:
            @pl.when(it == 0)
            def _():
                for cp in wo_copies:
                    cp.wait()

        out_project(h1, att1, (it if head else it - LAG,), False)

        if head:
            @pl.when(it < LAG - 1)
            def _():
                set_single_tokens(load_input(it + 1))

            @pl.when(it == LAG - 1)
            def _():
                ffn_only((0, 1), it == LAG - 1)
                x_rest.wait()
                mem1 = _load_tiles(h1, 0, dm_tiles, slice(0, n_mem))
                _store_operand(h2, 0, mem_rows, jnp.concatenate([mem1, mem0], axis=0))
                _store_operand(h2, 0, first_rows,
                               _layernorm(xin[LAG * seg:(LAG + 1) * seg, :].astype(F32)))
                _store_operand(h2, 0, second_rows, _layernorm(xs[0:seg, :]))
        else:
            k = it - n_seg

            @pl.when(k != 2)
            def _():
                ffn_only((jnp.where(k == 0, n_seg - 1, n_full + k - 1),
                          jnp.where(k == 0, n_full - 1, n_full + k)), None)

            @pl.when(k == 1)
            def _():
                out_mid.start()

            @pl.when(k < LAG - 1)
            def _():
                set_single_tokens(_layernorm(xs[rows(it + 1 - LAG), :]))

    def full_step(t, projected_ahead):
        ff_segs = (t - 1, jnp.where(t == LAG, LAG - 2, t - LAG - 1))
        ffn_norm(ff_segs)
        attend(h2, att2, 2, t - first_ahead if projected_ahead else None,
               [functools.partial(ffn_up, j) for j in ff_steps])
        out_project(h2, att2, (t, t - LAG), True)
        if not projected_ahead:
            _store_operand(h2, 0, first_rows, _layernorm(xin[rows(t + 1), :].astype(F32)))
        _store_operand(h2, 0, second_rows, _layernorm(xs[rows(t + 1 - LAG), :]))
        ffn_down(ff_segs)

    ff_steps = range(0, ff_tiles, FF_TILES)
    _store_operand(h1, 0, slice(0, n_mem), mem0)
    set_single_tokens(load_input(0))

    lax.fori_loop(0, LAG, lambda i, c: (single_step(i, True), c)[1], 0)
    lax.fori_loop(LAG, first_ahead, lambda t, c: (full_step(t, False), c)[1], 0)
    lax.fori_loop(first_ahead, n_seg, lambda t, c: (full_step(t, True), c)[1], 0)
    out_early.start()
    both = _load_tiles(h2, 0, dm_tiles, mem_rows).astype(F32)
    _store_operand(h1, 0, slice(0, n_mem), both[n_mem:])
    set_single_tokens(_load_tiles(h2, 0, dm_tiles, second_rows).astype(F32))
    lax.fori_loop(n_seg, n_seg + LAG, lambda i, c: (single_step(i, False), c)[1], 0)

    out_last.start()
    out_early.wait()
    out_mid.wait()
    out_last.wait()


@functools.partial(jax.jit, static_argnames=("A_seg_len",))
def pallas_interleave_layers__memory_aug_recurrent_mem_tr__glu_gated_geglu__prompt_kernel(
    A_x: jax.Array,
    A_mem0: jax.Array,
    A_Wq: jax.Array,
    A_Wk: jax.Array,
    A_Wv: jax.Array,
    A_Wo: jax.Array,
    A_seg_len: int,
    B_x: jax.Array,
    B_w_gate: jax.Array,
    B_w_up: jax.Array,
    B_w_down: jax.Array,
):
    del B_x
    b, s, dm = A_x.shape
    _, n_heads, dh = A_Wq.shape
    n_mem = A_mem0.shape[1]
    dff = B_w_gate.shape[1]
    seg = int(A_seg_len)
    n_seg = s // seg
    assert b == 1 and dh == LANES and n_seg * seg == s and n_mem == 8 and seg % 16 == 0
    assert LAG == 4 and n_seg > 2 * LAG + AHEAD + 1
    hd = n_heads * dh
    full = 2 * (n_mem + seg)

    def tiled(n_rows, n_cols, dtype=BF16):
        return pltpu.VMEM((n_cols // LANES, n_rows, LANES), dtype)

    any_spec = pl.BlockSpec(memory_space=pl.ANY)
    out = pl.pallas_call(
        functools.partial(_kernel, n_mem=n_mem, seg=seg, n_seg=n_seg),
        out_shape=jax.ShapeDtypeStruct((s, dm), A_x.dtype),
        in_specs=[any_spec, pl.BlockSpec(memory_space=pltpu.VMEM)] + [any_spec] * 7,
        out_specs=any_spec,
        scratch_shapes=[
            pltpu.VMEM((3 * n_heads, dm // LANES, LANES // 2, dh), jnp.uint32),
            tiled(hd, dm),
            tiled(dm, dff), tiled(dm, dff), tiled(dff, dm),
            pltpu.VMEM((dm // LANES, LANES * n_heads, dh), BF16),
            pltpu.VMEM((s, dm), BF16),
            pltpu.VMEM((s, dm), F32),
            pltpu.VMEM((s, dm), BF16),
            tiled(AHEAD * seg, dm),
            tiled(AHEAD * seg, 3 * hd, F32),
            tiled(full, dm), tiled(full, hd),
            tiled(full // 2, dm, F32), tiled(full // 2, hd, F32),
            tiled(2 * seg, dm), tiled(2 * seg, dff),
            pltpu.SemaphoreType.DMA((dm // LANES,)),
            pltpu.SemaphoreType.DMA((4,)),
            pltpu.SemaphoreType.DMA((3,)),
            pltpu.SemaphoreType.DMA((3,)),
        ],
        compiler_params=pltpu.CompilerParams(vmem_limit_bytes=110 * 1024 * 1024),
    )(
        A_x.reshape(s, dm),
        A_mem0.reshape(n_mem, dm),
        A_Wq.reshape(dm * n_heads, dh),
        A_Wk.reshape(dm * n_heads, dh),
        A_Wv.reshape(dm * n_heads, dh),
        A_Wo.reshape(hd, dm),
        B_w_gate,
        B_w_up,
        B_w_down,
    )
    return out.reshape(b, s, dm)
```

```python
import functools

import jax
import jax.numpy as jnp
import numpy as np
from jax import lax
import jax.experimental.pallas as pl
import jax.experimental.pallas.tpu as pltpu

F32 = jnp.float32
BF16 = jnp.bfloat16
LANES = 128
LAG = 4
AHEAD = 12
STREAM_CHUNKS = 2
HEAD_GROUP = 4
FF_TILES = 7
OUT_TILES = 4
EPS = 1e-5


def _layernorm(x):
    m = jnp.mean(x, axis=-1, keepdims=True)
    c = x - m
    v = jnp.mean(c * c, axis=-1, keepdims=True)
    return c * lax.rsqrt(v + EPS)


def _gelu(x):
    c = float(np.sqrt(2.0 / np.pi))
    return x * (0.5 * (1.0 + jnp.tanh(c * (x + 0.044715 * (x * x * x)))))


def _dot(a, b):
    return jnp.dot(a, b, preferred_element_type=F32)


def _dot_nt(a, b):
    return lax.dot_general(a, b, (((1,), (1,)), ((), ())), preferred_element_type=F32)


def _softmax(s):
    e = jnp.exp(s - jnp.max(s, axis=-1, keepdims=True))
    total = jnp.sum(e, axis=-1, keepdims=True)
    r = pl.reciprocal(total, approx=True)
    return e * (r * (2.0 - total * r))


def _score_mask(n_layers, n_mem, seg):
    n = n_layers * (n_mem + seg)

    def layer_and_pos(i):
        layer = jnp.zeros_like(i)
        pos = i
        for l in range(n_layers):
            in_mem = (i >= l * n_mem) & (i < (l + 1) * n_mem)
            lo = n_layers * n_mem + l * seg
            in_seg = (i >= lo) & (i < lo + seg)
            layer = jnp.where(in_mem | in_seg, l, layer)
            pos = jnp.where(in_mem, i - l * n_mem, jnp.where(in_seg, i - lo + n_mem, pos))
        return layer, pos

    r_layer, r_pos = layer_and_pos(lax.broadcasted_iota(jnp.int32, (n, n), 0))
    c_layer, c_pos = layer_and_pos(lax.broadcasted_iota(jnp.int32, (n, n), 1))
    same = r_layer == c_layer
    keep = same & ((r_pos < n_mem) | (r_pos >= c_pos))
    fill = jnp.where(same, -1e9, -jnp.inf).astype(F32)
    return keep, fill


def _load_tiles(ref, lo, n, rows=slice(None)):
    return jnp.concatenate([ref[t, rows, :] for t in range(lo, lo + n)], axis=1)


def _store_operand(ref, lo, rows, val):
    for t in range(val.shape[1] // LANES):
        tile = val[:, t * LANES:(t + 1) * LANES].astype(BF16)
        ref[lo + t, rows, :] = tile.astype(ref.dtype)


def _kernel(x_hbm, mem0_ref, wq_hbm, wk_hbm, wv_hbm, wo_hbm, wg_hbm, wu_hbm, wd_hbm,
            out_hbm,
            wqkv, wo, wg, wu, wd, stage, xin, xs, xout, ha, ahead, h2, att2, h1, att1, hf, act,
            stage_sem, w_sem, x_sem, out_sem, *, n_mem, seg, n_seg):
    n_heads, dm_tiles = wqkv.shape[0] // 3, wqkv.shape[1]
    dh = LANES
    ff_tiles = wg.shape[0]
    scale = float(dh) ** -0.5
    n_groups = n_heads // HEAD_GROUP
    every = slice(None)
    mem_rows = slice(0, 2 * n_mem)
    first_rows = slice(2 * n_mem, 2 * n_mem + seg)
    second_rows = slice(2 * n_mem + seg, 2 * n_mem + 2 * seg)
    first_ahead = n_seg - AHEAD

    def rows(s):
        if isinstance(s, int):
            return slice(s * seg, (s + 1) * seg)
        return pl.ds(pl.multiple_of(s * seg, seg), seg)

    def attend(h_ref, att, n_layers, ahead_seg=None, fillers=()):
        keep, fill = _score_mask(n_layers, n_mem, seg)
        fillers = list(fillers)

        def operand(x):
            return x.astype(BF16).astype(h_ref.dtype)

        def project(g):
            if ahead_seg is None:
                h = _load_tiles(h_ref, 0, dm_tiles)
            else:
                h = jnp.concatenate([_load_tiles(h_ref, 0, dm_tiles, mem_rows),
                                     _load_tiles(h_ref, 0, dm_tiles, second_rows)], axis=0)
            out = []
            for i in range(3):
                tile = i * n_heads + g * HEAD_GROUP
                w = [pltpu.bitcast(wqkv[tile + j].reshape(dm_tiles * LANES // 2, dh), BF16)
                     for j in range(HEAD_GROUP)]
                y = _dot(h, jnp.concatenate(w, axis=1))
                heads = [y[:, j * dh:(j + 1) * dh] for j in range(HEAD_GROUP)]
                if ahead_seg is not None:
                    heads = [jnp.concatenate([z[mem_rows], ahead[tile + j, rows(ahead_seg), :],
                                              z[2 * n_mem:]], axis=0)
                             for j, z in enumerate(heads)]
                out.append([operand(z) for z in heads])
            return out

        def mix(g, probs, v):
            for i in range(HEAD_GROUP):
                att[g * HEAD_GROUP + i] = operand(_dot(probs[i], v[i]))

        q, k, v = project(0)
        pending = None
        for g in range(n_groups):
            probs = [operand(_softmax(jnp.where(keep, _dot_nt(q[i], k[i]) * scale, fill)))
                     for i in range(HEAD_GROUP)]
            if pending is not None:
                mix(*pending)
            pending = (g, probs, v)
            if g + 1 < n_groups:
                q, k, v = project(g + 1)
            elif fillers:
                fillers.pop(0)()
        mix(*pending)
        for f in fillers:
            f()

    def out_project(h_ref, att, segs, first_from_input):
        n_rows = len(segs) * n_mem
        a = _load_tiles(att, 0, n_heads)
        for j in range(0, dm_tiles, OUT_TILES):
            cols = slice(j * LANES, (j + OUT_TILES) * LANES)
            o = _dot(a, _load_tiles(wo, j, OUT_TILES))
            _store_operand(h_ref, j, slice(0, n_rows), o[0:n_rows])
            for l, s in enumerate(segs):
                if first_from_input and l == 0:
                    x = xin[rows(s), cols].astype(F32)
                else:
                    x = xs[rows(s), cols]
                xs[rows(s), cols] = x + o[n_rows + l * seg:n_rows + (l + 1) * seg]

    def ffn_norm(segs):
        for l, s in enumerate(segs):
            _store_operand(hf, 0, slice(l * seg, (l + 1) * seg), _layernorm(xs[rows(s), :]))

    def ffn_up(j):
        h = _load_tiles(hf, 0, dm_tiles)
        g = _dot(h, _load_tiles(wg, j, FF_TILES))
        u = _dot(h, _load_tiles(wu, j, FF_TILES))
        _store_operand(act, j, every, _gelu(g) * u)

    def ffn_down(segs):
        a = _load_tiles(act, 0, ff_tiles)
        for j in range(0, dm_tiles, OUT_TILES):
            cols = slice(j * LANES, (j + OUT_TILES) * LANES)
            o = _dot(a, _load_tiles(wd, j, OUT_TILES))
            for l, s in enumerate(segs):
                y = xs[rows(s), cols] + o[l * seg:(l + 1) * seg]
                xs[rows(s), cols] = y
                xout[rows(s), cols] = y.astype(BF16)

    def load_input(s):
        x = xin[rows(s), :].astype(F32)
        xs[rows(s), :] = x
        return _layernorm(x)

    chunk_rows = LANES * n_heads

    def stage_copy(src, c):
        return pltpu.make_async_copy(
            src.at[pl.ds(pl.multiple_of(c * chunk_rows, chunk_rows), chunk_rows), :],
            stage.at[c], stage_sem.at[c])

    def tile_copies(src, dst, sem):
        return [pltpu.make_async_copy(src.at[:, t * LANES:(t + 1) * LANES], dst.at[t], sem)
                for t in range(dst.shape[0])]

    def row_copy(src, dst, lo, hi, sem):
        return pltpu.make_async_copy(
            src.at[lo * seg:hi * seg, :], dst.at[lo * seg:hi * seg, :], sem)

    x_ahead = row_copy(x_hbm, xin, first_ahead, n_seg, x_sem.at[0])
    x_head = row_copy(x_hbm, xin, 0, LAG + 1, x_sem.at[1])
    x_rest = row_copy(x_hbm, xin, LAG + 1, first_ahead, x_sem.at[2])
    wo_copies = tile_copies(wo_hbm, wo, w_sem.at[0])
    gate_copies = tile_copies(wg_hbm, wg, w_sem.at[1])
    up_copies = tile_copies(wu_hbm, wu, w_sem.at[2])
    down_copies = tile_copies(wd_hbm, wd, w_sem.at[3])
    n_full = n_seg - LAG
    out_early = row_copy(xout, out_hbm, 0, n_full - 1, out_sem.at[0])
    out_mid = row_copy(xout, out_hbm, n_full - 1, n_seg - 2, out_sem.at[1])
    out_last = row_copy(xout, out_hbm, n_seg - 2, n_seg, out_sem.at[2])

    x_ahead.start()
    for c in range(STREAM_CHUNKS):
        stage_copy(wq_hbm, c).start()

    x_ahead.wait()
    for c in range(STREAM_CHUNKS, dm_tiles):
        stage_copy(wq_hbm, c).start()
    x_head.start()
    for s in range(AHEAD):
        x = xin[(first_ahead + s) * seg:(first_ahead + s + 1) * seg, :].astype(F32)
        _store_operand(ha, 0, slice(s * seg, (s + 1) * seg), _layernorm(x))

    pairs = n_heads // 2

    def retile(which, cur_src, next_src, i):
        chunks = [i * STREAM_CHUNKS + j for j in range(STREAM_CHUNKS)]
        for c in chunks:
            stage_copy(cur_src, c).wait()
        words = stage.bitcast(jnp.uint32)
        h = jnp.concatenate([ha[c] for c in chunks], axis=1)
        for g in range(n_groups):
            columns = []
            for j in range(g * HEAD_GROUP // 2, (g + 1) * HEAD_GROUP // 2):
                packed = [words[c, pl.ds(j, LANES, stride=pairs), :] for c in chunks]
                for half in range(2):
                    tile = which * n_heads + 2 * j + half
                    w = [pltpu.bitcast((p >> (16 * half)).astype(jnp.uint16), BF16)
                         for p in packed]
                    for c, wc in zip(chunks, w):
                        wqkv[tile, c] = pltpu.bitcast(wc, jnp.uint32)
                    columns.append(jnp.concatenate(w, axis=0))
            y = _dot(h, jnp.concatenate(columns, axis=1))
            for j in range(HEAD_GROUP):
                tile = which * n_heads + g * HEAD_GROUP + j
                ahead[tile] = jnp.where(i == 0, 0.0, ahead[tile]) + y[:, j * dh:(j + 1) * dh]
        if next_src is not None:
            for c in chunks:
                stage_copy(next_src, c).start()
            t = which * n_iter + i
            pltpu.make_async_copy(wo_hbm.at[:, pl.ds(pl.multiple_of(t * LANES, LANES), LANES)],
                                  wo.at[t], w_sem.at[0]).start()
        else:
            for step, copies in ((0, gate_copies), (2, up_copies)):
                @pl.when(i == step)
                def _(copies=copies):
                    for cp in copies:
                        cp.start()

    sources = (wq_hbm, wk_hbm, wv_hbm, None)
    n_iter = dm_tiles // STREAM_CHUNKS
    assert 2 * n_iter == dm_tiles and n_iter > 2
    for which in range(3):
        body = functools.partial(retile, which, sources[which], sources[which + 1])
        lax.fori_loop(0, n_iter, lambda i, c: (body(i), c)[1], 0)
    for cp in down_copies:
        cp.start()
    x_rest.start()

    x_head.wait()
    mem0 = mem0_ref[...].astype(F32)

    def set_single_tokens(normed):
        _store_operand(h1, 0, slice(n_mem, n_mem + seg), normed)

    def ffn_only(segs, wait):
        if wait is not None:
            @pl.when(wait)
            def _():
                for cp in gate_copies + up_copies:
                    cp.wait()
        ffn_norm(segs)
        for j in ff_steps:
            ffn_up(j)
        if wait is not None:
            @pl.when(wait)
            def _():
                for cp in down_copies:
                    cp.wait()
        ffn_down(segs)

    def single_step(it, head):
        attend(h1, att1, 1)
        if head:
            set_single_tokens(load_input(it + 1))
        else:
            set_single_tokens(_layernorm(xs[rows(jnp.minimum(it + 1 - LAG, n_seg - 1)), :]))
        out_project(h1, att1, (it if head else it - LAG,), False)

        if head:
            @pl.when(it == LAG - 1)
            def _():
                ffn_only((0, 1), it == LAG - 1)
                x_rest.wait()
                mem1 = _load_tiles(h1, 0, dm_tiles, slice(0, n_mem))
                _store_operand(h2, 0, mem_rows, jnp.concatenate([mem1, mem0], axis=0))
                _store_operand(h2, 0, first_rows,
                               _layernorm(xin[LAG * seg:(LAG + 1) * seg, :].astype(F32)))
                _store_operand(h2, 0, second_rows, _layernorm(xs[0:seg, :]))
        else:
            k = it - n_seg

            @pl.when(k != 2)
            def _():
                ffn_only((jnp.where(k == 0, n_seg - 1, n_full + k - 1),
                          jnp.where(k == 0, n_full - 1, n_full + k)), None)

            @pl.when(k == 1)
            def _():
                out_mid.start()

    def full_step(t, projected_ahead):
        ff_segs = (t - 1, jnp.where(t == LAG, LAG - 2, t - LAG - 1))
        ffn_norm(ff_segs)
        attend(h2, att2, 2, t - first_ahead if projected_ahead else None,
               [functools.partial(ffn_up, j) for j in ff_steps])
        out_project(h2, att2, (t, t - LAG), True)
        if not projected_ahead:
            _store_operand(h2, 0, first_rows, _layernorm(xin[rows(t + 1), :].astype(F32)))
        _store_operand(h2, 0, second_rows, _layernorm(xs[rows(t + 1 - LAG), :]))
        ffn_down(ff_segs)

    ff_steps = range(0, ff_tiles, FF_TILES)
    _store_operand(h1, 0, slice(0, n_mem), mem0)
    set_single_tokens(load_input(0))

    for cp in wo_copies:
        cp.wait()
    lax.fori_loop(0, LAG, lambda i, c: (single_step(i, True), c)[1], 0)
    lax.fori_loop(LAG, first_ahead, lambda t, c: (full_step(t, False), c)[1], 0)
    lax.fori_loop(first_ahead, n_seg, lambda t, c: (full_step(t, True), c)[1], 0)
    out_early.start()
    both = _load_tiles(h2, 0, dm_tiles, mem_rows).astype(F32)
    _store_operand(h1, 0, slice(0, n_mem), both[n_mem:])
    set_single_tokens(_load_tiles(h2, 0, dm_tiles, second_rows).astype(F32))
    lax.fori_loop(n_seg, n_seg + LAG, lambda i, c: (single_step(i, False), c)[1], 0)

    out_last.start()
    out_early.wait()
    out_mid.wait()
    out_last.wait()


@functools.partial(jax.jit, static_argnames=("A_seg_len",))
def pallas_interleave_layers__memory_aug_recurrent_mem_tr__glu_gated_geglu__prompt_kernel(
    A_x: jax.Array,
    A_mem0: jax.Array,
    A_Wq: jax.Array,
    A_Wk: jax.Array,
    A_Wv: jax.Array,
    A_Wo: jax.Array,
    A_seg_len: int,
    B_x: jax.Array,
    B_w_gate: jax.Array,
    B_w_up: jax.Array,
    B_w_down: jax.Array,
):
    del B_x
    b, s, dm = A_x.shape
    _, n_heads, dh = A_Wq.shape
    n_mem = A_mem0.shape[1]
    dff = B_w_gate.shape[1]
    seg = int(A_seg_len)
    n_seg = s // seg
    assert b == 1 and dh == LANES and n_seg * seg == s and n_mem == 8 and seg % 16 == 0
    assert LAG == 4 and n_seg > 2 * LAG + AHEAD + 1
    hd = n_heads * dh
    full = 2 * (n_mem + seg)

    def tiled(n_rows, n_cols, dtype=BF16):
        return pltpu.VMEM((n_cols // LANES, n_rows, LANES), dtype)

    any_spec = pl.BlockSpec(memory_space=pl.ANY)
    out = pl.pallas_call(
        functools.partial(_kernel, n_mem=n_mem, seg=seg, n_seg=n_seg),
        out_shape=jax.ShapeDtypeStruct((s, dm), A_x.dtype),
        in_specs=[any_spec, pl.BlockSpec(memory_space=pltpu.VMEM)] + [any_spec] * 7,
        out_specs=any_spec,
        scratch_shapes=[
            pltpu.VMEM((3 * n_heads, dm // LANES, LANES // 2, dh), jnp.uint32),
            tiled(hd, dm),
            tiled(dm, dff), tiled(dm, dff), tiled(dff, dm),
            pltpu.VMEM((dm // LANES, LANES * n_heads, dh), BF16),
            pltpu.VMEM((s, dm), BF16),
            pltpu.VMEM((s, dm), F32),
            pltpu.VMEM((s, dm), BF16),
            tiled(AHEAD * seg, dm),
            tiled(AHEAD * seg, 3 * hd, F32),
            tiled(full, dm), tiled(full, hd),
            tiled(full // 2, dm, F32), tiled(full // 2, hd, F32),
            tiled(2 * seg, dm), tiled(2 * seg, dff),
            pltpu.SemaphoreType.DMA((dm // LANES,)),
            pltpu.SemaphoreType.DMA((4,)),
            pltpu.SemaphoreType.DMA((3,)),
            pltpu.SemaphoreType.DMA((3,)),
        ],
        compiler_params=pltpu.CompilerParams(vmem_limit_bytes=110 * 1024 * 1024),
    )(
        A_x.reshape(s, dm),
        A_mem0.reshape(n_mem, dm),
        A_Wq.reshape(dm * n_heads, dh),
        A_Wk.reshape(dm * n_heads, dh),
        A_Wv.reshape(dm * n_heads, dh),
        A_Wo.reshape(hd, dm),
        B_w_gate,
        B_w_up,
        B_w_down,
    )
    return out.reshape(b, s, dm)
```

```python
import functools

import jax
import jax.numpy as jnp
import numpy as np
from jax import lax
import jax.experimental.pallas as pl
import jax.experimental.pallas.tpu as pltpu

F32 = jnp.float32
BF16 = jnp.bfloat16
LANES = 128
LAG = 4
AHEAD = 12
STREAM_CHUNKS = 2
HEAD_GROUP = 4
FF_TILES = 7
OUT_TILES = 4
EPS = 1e-5


def _layernorm(x):
    m = jnp.mean(x, axis=-1, keepdims=True)
    c = x - m
    v = jnp.mean(c * c, axis=-1, keepdims=True)
    return c * lax.rsqrt(v + EPS)


def _gelu(x):
    c = float(np.sqrt(2.0 / np.pi))
    return x * (0.5 * (1.0 + jnp.tanh(c * (x + 0.044715 * (x * x * x)))))


def _dot(a, b):
    return jnp.dot(a, b, preferred_element_type=F32)


def _dot_nt(a, b):
    return lax.dot_general(a, b, (((1,), (1,)), ((), ())), preferred_element_type=F32)


def _softmax(s):
    e = jnp.exp(s - jnp.max(s, axis=-1, keepdims=True))
    total = jnp.sum(e, axis=-1, keepdims=True)
    r = pl.reciprocal(total, approx=True)
    return e * (r * (2.0 - total * r))


def _score_mask(n_layers, n_mem, seg):
    n = n_layers * (n_mem + seg)

    def layer_and_pos(i):
        layer = jnp.zeros_like(i)
        pos = i
        for l in range(n_layers):
            in_mem = (i >= l * n_mem) & (i < (l + 1) * n_mem)
            lo = n_layers * n_mem + l * seg
            in_seg = (i >= lo) & (i < lo + seg)
            layer = jnp.where(in_mem | in_seg, l, layer)
            pos = jnp.where(in_mem, i - l * n_mem, jnp.where(in_seg, i - lo + n_mem, pos))
        return layer, pos

    r_layer, r_pos = layer_and_pos(lax.broadcasted_iota(jnp.int32, (n, n), 0))
    c_layer, c_pos = layer_and_pos(lax.broadcasted_iota(jnp.int32, (n, n), 1))
    same = r_layer == c_layer
    keep = same & ((r_pos < n_mem) | (r_pos >= c_pos))
    fill = jnp.where(same, -1e9, -jnp.inf).astype(F32)
    return keep, fill


def _loop(lo, hi, body):
    lax.fori_loop(lo, hi, lambda i, carry: (body(i), carry)[1], 0)


def _load_tiles(ref, lo, n, rows=slice(None)):
    return jnp.concatenate([ref[t, rows, :] for t in range(lo, lo + n)], axis=1)


def _store_operand(ref, lo, rows, val):
    for t in range(val.shape[1] // LANES):
        tile = val[:, t * LANES:(t + 1) * LANES].astype(BF16)
        ref[lo + t, rows, :] = tile.astype(ref.dtype)


def _kernel(x_hbm, mem0_ref, wq_hbm, wk_hbm, wv_hbm, wo_hbm, wg_hbm, wu_hbm, wd_hbm,
            out_hbm,
            wqkv, wo, wg, wu, wd, stage, xin, xs, xout, ha, ahead, h2, att2, h1, att1, hf, act,
            stage_sem, w_sem, x_sem, out_sem, *, n_mem, seg, n_seg):
    n_heads, dm_tiles = wqkv.shape[0] // 3, wqkv.shape[1]
    dh = LANES
    ff_tiles = wg.shape[0]
    scale = float(dh) ** -0.5
    n_groups = n_heads // HEAD_GROUP
    every = slice(None)
    mem_rows = slice(0, 2 * n_mem)
    first_rows = slice(2 * n_mem, 2 * n_mem + seg)
    second_rows = slice(2 * n_mem + seg, 2 * n_mem + 2 * seg)
    first_ahead = n_seg - AHEAD

    def rows(s):
        if isinstance(s, int):
            return slice(s * seg, (s + 1) * seg)
        return pl.ds(pl.multiple_of(s * seg, seg), seg)

    def attend(h_ref, att, n_layers, ahead_seg=None, fillers=()):
        keep, fill = _score_mask(n_layers, n_mem, seg)
        fillers = list(fillers)

        def operand(x):
            return x.astype(BF16).astype(h_ref.dtype)

        def project(g):
            if ahead_seg is None:
                h = _load_tiles(h_ref, 0, dm_tiles)
            else:
                h = jnp.concatenate([_load_tiles(h_ref, 0, dm_tiles, mem_rows),
                                     _load_tiles(h_ref, 0, dm_tiles, second_rows)], axis=0)
            out = []
            for i in range(3):
                tile = i * n_heads + g * HEAD_GROUP
                w = [pltpu.bitcast(wqkv[tile + j].reshape(dm_tiles * LANES // 2, dh), BF16)
                     for j in range(HEAD_GROUP)]
                y = _dot(h, jnp.concatenate(w, axis=1))
                heads = [y[:, j * dh:(j + 1) * dh] for j in range(HEAD_GROUP)]
                if ahead_seg is not None:
                    heads = [jnp.concatenate([z[mem_rows], ahead[tile + j, rows(ahead_seg), :],
                                              z[2 * n_mem:]], axis=0)
                             for j, z in enumerate(heads)]
                out.append([operand(z) for z in heads])
            return out

        def mix(g, probs, v):
            for i in range(HEAD_GROUP):
                att[g * HEAD_GROUP + i] = operand(_dot(probs[i], v[i]))

        q, k, v = project(0)
        pending = None
        for g in range(n_groups):
            probs = [operand(_softmax(jnp.where(keep, _dot_nt(q[i], k[i]) * scale, fill)))
                     for i in range(HEAD_GROUP)]
            if pending is not None:
                mix(*pending)
            pending = (g, probs, v)
            if g + 1 < n_groups:
                q, k, v = project(g + 1)
            elif fillers:
                fillers.pop(0)()
        mix(*pending)
        for f in fillers:
            f()

    def out_project(h_ref, att, segs, first_from_input):
        n_rows = len(segs) * n_mem
        a = _load_tiles(att, 0, n_heads)
        for j in range(0, dm_tiles, OUT_TILES):
            cols = slice(j * LANES, (j + OUT_TILES) * LANES)
            o = _dot(a, _load_tiles(wo, j, OUT_TILES))
            _store_operand(h_ref, j, slice(0, n_rows), o[0:n_rows])
            for l, s in enumerate(segs):
                if first_from_input and l == 0:
                    x = xin[rows(s), cols].astype(F32)
                else:
                    x = xs[rows(s), cols]
                xs[rows(s), cols] = x + o[n_rows + l * seg:n_rows + (l + 1) * seg]

    def ffn_norm(segs):
        for l, s in enumerate(segs):
            _store_operand(hf, 0, slice(l * seg, (l + 1) * seg), _layernorm(xs[rows(s), :]))

    def ffn_up(j):
        h = _load_tiles(hf, 0, dm_tiles)
        g = _dot(h, _load_tiles(wg, j, FF_TILES))
        u = _dot(h, _load_tiles(wu, j, FF_TILES))
        _store_operand(act, j, every, _gelu(g) * u)

    def ffn_down(segs):
        a = _load_tiles(act, 0, ff_tiles)
        for j in range(0, dm_tiles, OUT_TILES):
            cols = slice(j * LANES, (j + OUT_TILES) * LANES)
            o = _dot(a, _load_tiles(wd, j, OUT_TILES))
            for l, s in enumerate(segs):
                y = xs[rows(s), cols] + o[l * seg:(l + 1) * seg]
                xs[rows(s), cols] = y
                xout[rows(s), cols] = y.astype(BF16)

    def load_input(s):
        x = xin[rows(s), :].astype(F32)
        xs[rows(s), :] = x
        return _layernorm(x)

    chunk_rows = LANES * n_heads

    def stage_copy(src, c):
        return pltpu.make_async_copy(
            src.at[pl.ds(pl.multiple_of(c * chunk_rows, chunk_rows), chunk_rows), :],
            stage.at[c], stage_sem.at[c])

    def tile_copies(src, dst, sem):
        return [pltpu.make_async_copy(src.at[:, t * LANES:(t + 1) * LANES], dst.at[t], sem)
                for t in range(dst.shape[0])]

    def row_copy(src, dst, lo, hi, sem):
        return pltpu.make_async_copy(
            src.at[lo * seg:hi * seg, :], dst.at[lo * seg:hi * seg, :], sem)

    x_ahead = row_copy(x_hbm, xin, first_ahead, n_seg, x_sem.at[0])
    x_head = row_copy(x_hbm, xin, 0, LAG + 1, x_sem.at[1])
    x_rest = row_copy(x_hbm, xin, LAG + 1, first_ahead, x_sem.at[2])
    wo_copies = tile_copies(wo_hbm, wo, w_sem.at[0])
    gate_copies = tile_copies(wg_hbm, wg, w_sem.at[1])
    up_copies = tile_copies(wu_hbm, wu, w_sem.at[2])
    down_copies = tile_copies(wd_hbm, wd, w_sem.at[3])
    n_full = n_seg - LAG
    out_early = row_copy(xout, out_hbm, 0, n_full - 1, out_sem.at[0])
    out_mid = row_copy(xout, out_hbm, n_full - 1, n_seg - 2, out_sem.at[1])
    out_last = row_copy(xout, out_hbm, n_seg - 2, n_seg, out_sem.at[2])

    x_ahead.start()
    stage_copy(wq_hbm, 0).start()
    x_ahead.wait()
    for c in range(1, 3):
        stage_copy(wq_hbm, c).start()
    for s in range(AHEAD):
        x = xin[(first_ahead + s) * seg:(first_ahead + s + 1) * seg, :].astype(F32)
        _store_operand(ha, 0, slice(s * seg, (s + 1) * seg), _layernorm(x))

    pairs = n_heads // 2

    def retile(which, chunks):
        for c in chunks:
            pltpu.make_async_copy(stage.at[c], stage.at[c], stage_sem.at[c]).wait()
        words = stage.bitcast(jnp.uint32)
        h = jnp.concatenate([ha[c] for c in chunks], axis=1)
        for g in range(n_groups):
            columns = []
            for j in range(g * HEAD_GROUP // 2, (g + 1) * HEAD_GROUP // 2):
                packed = [words[c, pl.ds(j, LANES, stride=pairs), :] for c in chunks]
                for half in range(2):
                    tile = which * n_heads + 2 * j + half
                    w = [pltpu.bitcast((p >> (16 * half)).astype(jnp.uint16), BF16)
                         for p in packed]
                    for c, wc in zip(chunks, w):
                        wqkv[tile, c] = pltpu.bitcast(wc, jnp.uint32)
                    columns.append(jnp.concatenate(w, axis=0))
            y = _dot(h, jnp.concatenate(columns, axis=1))
            for j in range(HEAD_GROUP):
                tile = which * n_heads + g * HEAD_GROUP + j
                old = jnp.where(chunks[0] == 0, 0.0, ahead[tile])
                ahead[tile] = old + y[:, j * dh:(j + 1) * dh]

    def stream_first(c):
        retile(0, [c])
        stage_copy(wk_hbm, c).start()

    def stream(n):
        which = n // n_iter
        chunks = [(n % n_iter) * STREAM_CHUNKS + j for j in range(STREAM_CHUNKS)]
        retile(which, chunks)
        for w, src in enumerate((wk_hbm, wv_hbm)):
            @pl.when(which == w)
            def _(src=src):
                for c in chunks:
                    stage_copy(src, c).start()

        @pl.when(which < 2)
        def _():
            cols = pl.ds(pl.multiple_of(n * LANES, LANES), LANES)
            pltpu.make_async_copy(wo_hbm.at[:, cols], wo.at[n], w_sem.at[0]).start()

        for step, copies in ((0, gate_copies), (2, up_copies)):
            @pl.when(n == 2 * n_iter + step)
            def _(copies=copies):
                for cp in copies:
                    cp.start()

    n_iter = dm_tiles // STREAM_CHUNKS
    assert 2 * n_iter == dm_tiles and n_iter > 2
    for c in range(3, dm_tiles):
        stage_copy(wq_hbm, c).start()
    x_head.start()
    _loop(0, STREAM_CHUNKS, stream_first)
    wo_copies[0].start()
    _loop(1, 3 * n_iter, stream)
    for cp in down_copies:
        cp.start()
    x_rest.start()

    x_head.wait()
    mem0 = mem0_ref[...].astype(F32)

    def ffn_only(segs):
        ffn_norm(segs)
        for j in ff_steps:
            ffn_up(j)
        ffn_down(segs)

    def single_step(s, next_tokens):
        attend(h1, att1, 1)
        _store_operand(h1, 0, slice(n_mem, n_mem + seg), next_tokens())
        out_project(h1, att1, (s,), False)

    def head_step(s):
        single_step(s, lambda: load_input(s + 1))

        @pl.when(s == LAG - 1)
        def _():
            for cp in gate_copies + up_copies + down_copies + [x_rest]:
                cp.wait()
            ffn_only((0, 1))
            mem1 = _load_tiles(h1, 0, dm_tiles, slice(0, n_mem))
            _store_operand(h2, 0, mem_rows, jnp.concatenate([mem1, mem0], axis=0))
            _store_operand(h2, 0, first_rows, _layernorm(xin[rows(LAG), :].astype(F32)))
            _store_operand(h2, 0, second_rows, _layernorm(xs[rows(0), :]))

    def tail_step(k):
        s = n_full + k
        single_step(s, lambda: _layernorm(xs[rows(jnp.minimum(s + 1, n_seg - 1)), :]))

        @pl.when(k != 2)
        def _():
            ffn_only((jnp.where(k == 0, n_seg - 1, s - 1), jnp.where(k == 0, n_full - 1, s)))

        pl.when(k == 1)(out_mid.start)

    def full_step(t, projected_ahead):
        ff_segs = (t - 1, jnp.where(t == LAG, LAG - 2, t - LAG - 1))
        ffn_norm(ff_segs)
        attend(h2, att2, 2, t - first_ahead if projected_ahead else None,
               [functools.partial(ffn_up, j) for j in ff_steps])
        out_project(h2, att2, (t, t - LAG), True)
        if not projected_ahead:
            _store_operand(h2, 0, first_rows, _layernorm(xin[rows(t + 1), :].astype(F32)))
        _store_operand(h2, 0, second_rows, _layernorm(xs[rows(t + 1 - LAG), :]))
        ffn_down(ff_segs)

    ff_steps = range(0, ff_tiles, FF_TILES)
    _store_operand(h1, 0, slice(0, n_mem), mem0)
    _store_operand(h1, 0, slice(n_mem, n_mem + seg), load_input(0))

    for cp in wo_copies:
        cp.wait()
    _loop(0, LAG, head_step)
    _loop(LAG, first_ahead, lambda t: full_step(t, False))
    _loop(first_ahead, n_seg, lambda t: full_step(t, True))

    out_early.start()
    both = _load_tiles(h2, 0, dm_tiles, mem_rows).astype(F32)
    _store_operand(h1, 0, slice(0, n_mem), both[n_mem:])
    _store_operand(h1, 0, slice(n_mem, n_mem + seg),
                   _load_tiles(h2, 0, dm_tiles, second_rows).astype(F32))
    _loop(0, LAG, tail_step)

    out_last.start()
    out_early.wait()
    out_mid.wait()
    out_last.wait()


@functools.partial(jax.jit, static_argnames=("A_seg_len",))
def pallas_interleave_layers__memory_aug_recurrent_mem_tr__glu_gated_geglu__prompt_kernel(
    A_x: jax.Array,
    A_mem0: jax.Array,
    A_Wq: jax.Array,
    A_Wk: jax.Array,
    A_Wv: jax.Array,
    A_Wo: jax.Array,
    A_seg_len: int,
    B_x: jax.Array,
    B_w_gate: jax.Array,
    B_w_up: jax.Array,
    B_w_down: jax.Array,
):
    del B_x
    b, s, dm = A_x.shape
    _, n_heads, dh = A_Wq.shape
    n_mem = A_mem0.shape[1]
    dff = B_w_gate.shape[1]
    seg = int(A_seg_len)
    n_seg = s // seg
    assert b == 1 and dh == LANES and n_seg * seg == s and n_mem == 8 and seg % 16 == 0
    assert LAG == 4 and n_seg > 2 * LAG + AHEAD + 1
    hd = n_heads * dh
    full = 2 * (n_mem + seg)

    def tiled(n_rows, n_cols, dtype=BF16):
        return pltpu.VMEM((n_cols // LANES, n_rows, LANES), dtype)

    any_spec = pl.BlockSpec(memory_space=pl.ANY)
    out = pl.pallas_call(
        functools.partial(_kernel, n_mem=n_mem, seg=seg, n_seg=n_seg),
        out_shape=jax.ShapeDtypeStruct((s, dm), A_x.dtype),
        in_specs=[any_spec, pl.BlockSpec(memory_space=pltpu.VMEM)] + [any_spec] * 7,
        out_specs=any_spec,
        scratch_shapes=[
            pltpu.VMEM((3 * n_heads, dm // LANES, LANES // 2, dh), jnp.uint32),
            tiled(hd, dm),
            tiled(dm, dff), tiled(dm, dff), tiled(dff, dm),
            pltpu.VMEM((dm // LANES, LANES * n_heads, dh), BF16),
            pltpu.VMEM((s, dm), BF16),
            pltpu.VMEM((s, dm), F32),
            pltpu.VMEM((s, dm), BF16),
            tiled(AHEAD * seg, dm),
            tiled(AHEAD * seg, 3 * hd, F32),
            tiled(full, dm), tiled(full, hd),
            tiled(full // 2, dm, F32), tiled(full // 2, hd, F32),
            tiled(2 * seg, dm), tiled(2 * seg, dff),
            pltpu.SemaphoreType.DMA((dm // LANES,)),
            pltpu.SemaphoreType.DMA((4,)),
            pltpu.SemaphoreType.DMA((3,)),
            pltpu.SemaphoreType.DMA((3,)),
        ],
        compiler_params=pltpu.CompilerParams(vmem_limit_bytes=110 * 1024 * 1024),
    )(
        A_x.reshape(s, dm),
        A_mem0.reshape(n_mem, dm),
        A_Wq.reshape(dm * n_heads, dh),
        A_Wk.reshape(dm * n_heads, dh),
        A_Wv.reshape(dm * n_heads, dh),
        A_Wo.reshape(hd, dm),
        B_w_gate,
        B_w_up,
        B_w_down,
    )
    return out.reshape(b, s, dm)
```

```python
import functools

import jax
import jax.numpy as jnp
import numpy as np
from jax import lax
import jax.experimental.pallas as pl
import jax.experimental.pallas.tpu as pltpu

F32 = jnp.float32
BF16 = jnp.bfloat16
LANES = 128
LAG = 4
AHEAD = 13
STREAM_CHUNKS = 2
HEAD_GROUP = 4
FF_TILES = 7
OUT_TILES = 4
EPS = 1e-5


def _layernorm(x):
    m = jnp.mean(x, axis=-1, keepdims=True)
    c = x - m
    v = jnp.mean(c * c, axis=-1, keepdims=True)
    return c * lax.rsqrt(v + EPS)


def _gelu(x):
    c = float(np.sqrt(2.0 / np.pi))
    return x * (0.5 * (1.0 + jnp.tanh(c * (x + 0.044715 * (x * x * x)))))


def _dot(a, b):
    return jnp.dot(a, b, preferred_element_type=F32)


def _dot_nt(a, b):
    return lax.dot_general(a, b, (((1,), (1,)), ((), ())), preferred_element_type=F32)


def _softmax(s):
    e = jnp.exp(s - jnp.max(s, axis=-1, keepdims=True))
    total = jnp.sum(e, axis=-1, keepdims=True)
    r = pl.reciprocal(total, approx=True)
    return e * (r * (2.0 - total * r))


def _score_mask(n_layers, n_mem, seg):
    n = n_layers * (n_mem + seg)

    def layer_and_pos(i):
        layer = jnp.zeros_like(i)
        pos = i
        for l in range(n_layers):
            in_mem = (i >= l * n_mem) & (i < (l + 1) * n_mem)
            lo = n_layers * n_mem + l * seg
            in_seg = (i >= lo) & (i < lo + seg)
            layer = jnp.where(in_mem | in_seg, l, layer)
            pos = jnp.where(in_mem, i - l * n_mem, jnp.where(in_seg, i - lo + n_mem, pos))
        return layer, pos

    r_layer, r_pos = layer_and_pos(lax.broadcasted_iota(jnp.int32, (n, n), 0))
    c_layer, c_pos = layer_and_pos(lax.broadcasted_iota(jnp.int32, (n, n), 1))
    same = r_layer == c_layer
    keep = same & ((r_pos < n_mem) | (r_pos >= c_pos))
    fill = jnp.where(same, -1e9, -jnp.inf).astype(F32)
    return keep, fill


def _loop(lo, hi, body):
    lax.fori_loop(lo, hi, lambda i, carry: (body(i), carry)[1], 0)


def _load_tiles(ref, lo, n, rows=slice(None)):
    return jnp.concatenate([ref[t, rows, :] for t in range(lo, lo + n)], axis=1)


def _store_operand(ref, lo, rows, val):
    for t in range(val.shape[1] // LANES):
        tile = val[:, t * LANES:(t + 1) * LANES].astype(BF16)
        ref[lo + t, rows, :] = tile.astype(ref.dtype)


def _kernel(x_hbm, mem0_ref, wq_hbm, wk_hbm, wv_hbm, wo_hbm, wg_hbm, wu_hbm, wd_hbm,
            out_hbm,
            wqkv, wo, wg, wu, wd, stage, xin, xs, xout, ha, ahead, h2, att2, h1, att1, hf, act,
            stage_sem, w_sem, x_sem, out_sem, *, n_mem, seg, n_seg):
    n_heads, dm_tiles = wqkv.shape[0] // 3, wqkv.shape[1]
    dh = LANES
    ff_tiles = wg.shape[0]
    scale = float(dh) ** -0.5
    n_groups = n_heads // HEAD_GROUP
    every = slice(None)
    mem_rows = slice(0, 2 * n_mem)
    first_rows = slice(2 * n_mem, 2 * n_mem + seg)
    second_rows = slice(2 * n_mem + seg, 2 * n_mem + 2 * seg)
    first_ahead = n_seg - AHEAD

    def rows(s):
        if isinstance(s, int):
            return slice(s * seg, (s + 1) * seg)
        return pl.ds(pl.multiple_of(s * seg, seg), seg)

    def attend(h_ref, att, n_layers, ahead_seg=None, fillers=()):
        keep, fill = _score_mask(n_layers, n_mem, seg)
        fillers = list(fillers)

        def operand(x):
            return x.astype(BF16).astype(h_ref.dtype)

        def project(g):
            if ahead_seg is None:
                h = _load_tiles(h_ref, 0, dm_tiles)
            else:
                h = jnp.concatenate([_load_tiles(h_ref, 0, dm_tiles, mem_rows),
                                     _load_tiles(h_ref, 0, dm_tiles, second_rows)], axis=0)
            out = []
            for i in range(3):
                tile = i * n_heads + g * HEAD_GROUP
                w = [pltpu.bitcast(wqkv[tile + j].reshape(dm_tiles * LANES // 2, dh), BF16)
                     for j in range(HEAD_GROUP)]
                y = _dot(h, jnp.concatenate(w, axis=1))
                heads = [y[:, j * dh:(j + 1) * dh] for j in range(HEAD_GROUP)]
                if ahead_seg is not None:
                    heads = [jnp.concatenate([z[mem_rows], ahead[tile + j, rows(ahead_seg), :],
                                              z[2 * n_mem:]], axis=0)
                             for j, z in enumerate(heads)]
                out.append([operand(z) for z in heads])
            return out

        def mix(g, probs, v):
            for i in range(HEAD_GROUP):
                att[g * HEAD_GROUP + i] = operand(_dot(probs[i], v[i]))

        q, k, v = project(0)
        pending = None
        for g in range(n_groups):
            probs = [operand(_softmax(jnp.where(keep, _dot_nt(q[i], k[i]) * scale, fill)))
                     for i in range(HEAD_GROUP)]
            if pending is not None:
                mix(*pending)
            pending = (g, probs, v)
            if g + 1 < n_groups:
                q, k, v = project(g + 1)
            elif fillers:
                fillers.pop(0)()
        mix(*pending)
        for f in fillers:
            f()

    def out_project(h_ref, att, segs, first_from_input):
        n_rows = len(segs) * n_mem
        a = _load_tiles(att, 0, n_heads)
        for j in range(0, dm_tiles, OUT_TILES):
            cols = slice(j * LANES, (j + OUT_TILES) * LANES)
            o = _dot(a, _load_tiles(wo, j, OUT_TILES))
            _store_operand(h_ref, j, slice(0, n_rows), o[0:n_rows])
            for l, s in enumerate(segs):
                if first_from_input and l == 0:
                    x = xin[rows(s), cols].astype(F32)
                else:
                    x = xs[rows(s), cols]
                xs[rows(s), cols] = x + o[n_rows + l * seg:n_rows + (l + 1) * seg]

    def ffn_norm(segs):
        for l, s in enumerate(segs):
            _store_operand(hf, 0, slice(l * seg, (l + 1) * seg), _layernorm(xs[rows(s), :]))

    def ffn_up(j):
        h = _load_tiles(hf, 0, dm_tiles)
        g = _dot(h, _load_tiles(wg, j, FF_TILES))
        u = _dot(h, _load_tiles(wu, j, FF_TILES))
        _store_operand(act, j, every, _gelu(g) * u)

    def ffn_down(segs):
        a = _load_tiles(act, 0, ff_tiles)
        for j in range(0, dm_tiles, OUT_TILES):
            cols = slice(j * LANES, (j + OUT_TILES) * LANES)
            o = _dot(a, _load_tiles(wd, j, OUT_TILES))
            for l, s in enumerate(segs):
                y = xs[rows(s), cols] + o[l * seg:(l + 1) * seg]
                xs[rows(s), cols] = y
                xout[rows(s), cols] = y.astype(BF16)

    def load_input(s):
        x = xin[rows(s), :].astype(F32)
        xs[rows(s), :] = x
        return _layernorm(x)

    chunk_rows = LANES * n_heads

    def stage_copy(src, c):
        return pltpu.make_async_copy(
            src.at[pl.ds(pl.multiple_of(c * chunk_rows, chunk_rows), chunk_rows), :],
            stage.at[c], stage_sem.at[c])

    def tile_copy(src, dst, t, sem):
        start = t * LANES if isinstance(t, int) else pl.multiple_of(t * LANES, LANES)
        return pltpu.make_async_copy(src.at[:, pl.ds(start, LANES)], dst.at[t], sem)

    def start_tiles(src, dst, sem):
        for t in range(dst.shape[0]):
            tile_copy(src, dst, t, sem).start()

    def wait_filled(buf, sem):
        pltpu.make_async_copy(buf, buf, sem).wait()

    def row_copy(src, dst, lo, hi, sem):
        return pltpu.make_async_copy(
            src.at[lo * seg:hi * seg, :], dst.at[lo * seg:hi * seg, :], sem)

    x_ahead = row_copy(x_hbm, xin, first_ahead, n_seg, x_sem.at[0])
    x_head = row_copy(x_hbm, xin, 0, LAG + 1, x_sem.at[1])
    x_rest = row_copy(x_hbm, xin, LAG + 1, first_ahead, x_sem.at[2])
    n_full = n_seg - LAG
    out_early = row_copy(xout, out_hbm, 0, n_full - 1, out_sem.at[0])
    out_mid = row_copy(xout, out_hbm, n_full - 1, n_seg - 2, out_sem.at[1])
    out_last = row_copy(xout, out_hbm, n_seg - 2, n_seg, out_sem.at[2])

    x_ahead.start()
    stage_copy(wq_hbm, 0).start()
    x_ahead.wait()
    for c in range(1, 3):
        stage_copy(wq_hbm, c).start()
    for s in range(AHEAD):
        x = xin[(first_ahead + s) * seg:(first_ahead + s + 1) * seg, :].astype(F32)
        _store_operand(ha, 0, slice(s * seg, (s + 1) * seg), _layernorm(x))

    pairs = n_heads // 2

    def retile(which, chunks):
        for c in chunks:
            pltpu.make_async_copy(stage.at[c], stage.at[c], stage_sem.at[c]).wait()
        words = stage.bitcast(jnp.uint32)
        h = jnp.concatenate([ha[c] for c in chunks], axis=1)
        for g in range(n_groups):
            columns = []
            for j in range(g * HEAD_GROUP // 2, (g + 1) * HEAD_GROUP // 2):
                packed = [words[c, pl.ds(j, LANES, stride=pairs), :] for c in chunks]
                for half in range(2):
                    tile = which * n_heads + 2 * j + half
                    w = [pltpu.bitcast((p >> (16 * half)).astype(jnp.uint16), BF16)
                         for p in packed]
                    for c, wc in zip(chunks, w):
                        wqkv[tile, c] = pltpu.bitcast(wc, jnp.uint32)
                    columns.append(jnp.concatenate(w, axis=0))
            y = _dot(h, jnp.concatenate(columns, axis=1))
            for j in range(HEAD_GROUP):
                tile = which * n_heads + g * HEAD_GROUP + j
                old = jnp.where(chunks[0] == 0, 0.0, ahead[tile])
                ahead[tile] = old + y[:, j * dh:(j + 1) * dh]

    def stream_first(c):
        retile(0, [c])
        stage_copy(wk_hbm, c).start()

    def stream(n):
        which = n // n_iter
        chunks = [(n % n_iter) * STREAM_CHUNKS + j for j in range(STREAM_CHUNKS)]
        retile(which, chunks)
        for w, src in enumerate((wk_hbm, wv_hbm)):
            @pl.when(which == w)
            def _(src=src):
                for c in chunks:
                    stage_copy(src, c).start()

        @pl.when(which < 2)
        def _():
            tile_copy(wo_hbm, wo, n, w_sem.at[0]).start()

        pl.when(n == 2 * n_iter)(lambda: start_tiles(wg_hbm, wg, w_sem.at[1]))
        pl.when(n == 2 * n_iter + 2)(lambda: start_tiles(wu_hbm, wu, w_sem.at[2]))

    n_iter = dm_tiles // STREAM_CHUNKS
    assert 2 * n_iter == dm_tiles and n_iter > 2
    for c in range(3, dm_tiles):
        stage_copy(wq_hbm, c).start()
    x_head.start()
    _loop(0, STREAM_CHUNKS, stream_first)
    tile_copy(wo_hbm, wo, 0, w_sem.at[0]).start()
    _loop(1, 3 * n_iter, stream)
    start_tiles(wd_hbm, wd, w_sem.at[3])
    x_rest.start()

    x_head.wait()
    mem0 = mem0_ref[...].astype(F32)

    def ffn_only(segs):
        ffn_norm(segs)
        for j in ff_steps:
            ffn_up(j)
        ffn_down(segs)

    def single_step(s, next_tokens):
        attend(h1, att1, 1)
        _store_operand(h1, 0, slice(n_mem, n_mem + seg), next_tokens())
        out_project(h1, att1, (s,), False)

    def head_step(s):
        single_step(s, lambda: load_input(s + 1))

        @pl.when(s == LAG - 1)
        def _():
            for i, w in enumerate((wg, wu, wd)):
                wait_filled(w, w_sem.at[1 + i])
            x_rest.wait()
            ffn_only((0, 1))
            mem1 = _load_tiles(h1, 0, dm_tiles, slice(0, n_mem))
            _store_operand(h2, 0, mem_rows, jnp.concatenate([mem1, mem0], axis=0))
            _store_operand(h2, 0, first_rows, _layernorm(xin[rows(LAG), :].astype(F32)))
            _store_operand(h2, 0, second_rows, _layernorm(xs[rows(0), :]))

    def tail_step(k):
        s = n_full + k
        single_step(s, lambda: _layernorm(xs[rows(jnp.minimum(s + 1, n_seg - 1)), :]))

        @pl.when(k != 2)
        def _():
            ffn_only((jnp.where(k == 0, n_seg - 1, s - 1), jnp.where(k == 0, n_full - 1, s)))

        pl.when(k == 1)(out_mid.start)

    def full_step(t, projected_ahead):
        ff_segs = (t - 1, jnp.where(t == LAG, LAG - 2, t - LAG - 1))
        ffn_norm(ff_segs)
        attend(h2, att2, 2, t - first_ahead if projected_ahead else None,
               [functools.partial(ffn_up, j) for j in ff_steps])
        out_project(h2, att2, (t, t - LAG), True)
        if not projected_ahead:
            _store_operand(h2, 0, first_rows, _layernorm(xin[rows(t + 1), :].astype(F32)))
        _store_operand(h2, 0, second_rows, _layernorm(xs[rows(t + 1 - LAG), :]))
        ffn_down(ff_segs)

    ff_steps = range(0, ff_tiles, FF_TILES)
    _store_operand(h1, 0, slice(0, n_mem), mem0)
    _store_operand(h1, 0, slice(n_mem, n_mem + seg), load_input(0))

    wait_filled(wo, w_sem.at[0])
    _loop(0, LAG, head_step)
    _loop(LAG, first_ahead, lambda t: full_step(t, False))
    _loop(first_ahead, n_seg, lambda t: full_step(t, True))

    out_early.start()
    both = _load_tiles(h2, 0, dm_tiles, mem_rows).astype(F32)
    _store_operand(h1, 0, slice(0, n_mem), both[n_mem:])
    _store_operand(h1, 0, slice(n_mem, n_mem + seg),
                   _load_tiles(h2, 0, dm_tiles, second_rows).astype(F32))
    _loop(0, LAG, tail_step)

    out_last.start()
    out_early.wait()
    out_mid.wait()
    out_last.wait()


@functools.partial(jax.jit, static_argnames=("A_seg_len",))
def pallas_interleave_layers__memory_aug_recurrent_mem_tr__glu_gated_geglu__prompt_kernel(
    A_x: jax.Array,
    A_mem0: jax.Array,
    A_Wq: jax.Array,
    A_Wk: jax.Array,
    A_Wv: jax.Array,
    A_Wo: jax.Array,
    A_seg_len: int,
    B_x: jax.Array,
    B_w_gate: jax.Array,
    B_w_up: jax.Array,
    B_w_down: jax.Array,
):
    del B_x
    b, s, dm = A_x.shape
    _, n_heads, dh = A_Wq.shape
    n_mem = A_mem0.shape[1]
    dff = B_w_gate.shape[1]
    seg = int(A_seg_len)
    n_seg = s // seg
    assert b == 1 and dh == LANES and n_seg * seg == s and n_mem == 8 and seg % 16 == 0
    assert LAG == 4 and n_seg > 2 * LAG + AHEAD + 1
    hd = n_heads * dh
    full = 2 * (n_mem + seg)

    def tiled(n_rows, n_cols, dtype=BF16):
        return pltpu.VMEM((n_cols // LANES, n_rows, LANES), dtype)

    any_spec = pl.BlockSpec(memory_space=pl.ANY)
    out = pl.pallas_call(
        functools.partial(_kernel, n_mem=n_mem, seg=seg, n_seg=n_seg),
        out_shape=jax.ShapeDtypeStruct((s, dm), A_x.dtype),
        in_specs=[any_spec, pl.BlockSpec(memory_space=pltpu.VMEM)] + [any_spec] * 7,
        out_specs=any_spec,
        scratch_shapes=[
            pltpu.VMEM((3 * n_heads, dm // LANES, LANES // 2, dh), jnp.uint32),
            tiled(hd, dm),
            tiled(dm, dff), tiled(dm, dff), tiled(dff, dm),
            pltpu.VMEM((dm // LANES, LANES * n_heads, dh), BF16),
            pltpu.VMEM((s, dm), BF16),
            pltpu.VMEM((s, dm), F32),
            pltpu.VMEM((s, dm), BF16),
            tiled(AHEAD * seg, dm),
            tiled(AHEAD * seg, 3 * hd, F32),
            tiled(full, dm), tiled(full, hd),
            tiled(full // 2, dm, F32), tiled(full // 2, hd, F32),
            tiled(2 * seg, dm), tiled(2 * seg, dff),
            pltpu.SemaphoreType.DMA((dm // LANES,)),
            pltpu.SemaphoreType.DMA((4,)),
            pltpu.SemaphoreType.DMA((3,)),
            pltpu.SemaphoreType.DMA((3,)),
        ],
        compiler_params=pltpu.CompilerParams(vmem_limit_bytes=110 * 1024 * 1024),
    )(
        A_x.reshape(s, dm),
        A_mem0.reshape(n_mem, dm),
        A_Wq.reshape(dm * n_heads, dh),
        A_Wk.reshape(dm * n_heads, dh),
        A_Wv.reshape(dm * n_heads, dh),
        A_Wo.reshape(hd, dm),
        B_w_gate,
        B_w_up,
        B_w_down,
    )
    return out.reshape(b, s, dm)
```

```python
import functools

import jax
import jax.numpy as jnp
import numpy as np
from jax import lax
import jax.experimental.pallas as pl
import jax.experimental.pallas.tpu as pltpu

F32 = jnp.float32
BF16 = jnp.bfloat16
LANES = 128
LAG = 4
AHEAD = 13
STREAM_CHUNKS = 2
HEAD_GROUP = 4
FF_TILES = 7
OUT_TILES = 4
EPS = 1e-5


def _layernorm(x):
    m = jnp.mean(x, axis=-1, keepdims=True)
    c = x - m
    v = jnp.mean(c * c, axis=-1, keepdims=True)
    return c * lax.rsqrt(v + EPS)


def _gelu(x):
    c = float(np.sqrt(2.0 / np.pi))
    return x * (0.5 * (1.0 + jnp.tanh(c * (x + 0.044715 * (x * x * x)))))


def _dot(a, b):
    return jnp.dot(a, b, preferred_element_type=F32)


def _dot_nt(a, b):
    return lax.dot_general(a, b, (((1,), (1,)), ((), ())), preferred_element_type=F32)


def _softmax(s):
    e = jnp.exp(s - jnp.max(s, axis=-1, keepdims=True))
    total = jnp.sum(e, axis=-1, keepdims=True)
    r = pl.reciprocal(total, approx=True)
    return e * (r * (2.0 - total * r))


def _score_mask(n_layers, n_mem, seg):
    n = n_layers * (n_mem + seg)

    def layer_and_pos(i):
        layer = jnp.zeros_like(i)
        pos = i
        for l in range(n_layers):
            in_mem = (i >= l * n_mem) & (i < (l + 1) * n_mem)
            lo = n_layers * n_mem + l * seg
            in_seg = (i >= lo) & (i < lo + seg)
            layer = jnp.where(in_mem | in_seg, l, layer)
            pos = jnp.where(in_mem, i - l * n_mem, jnp.where(in_seg, i - lo + n_mem, pos))
        return layer, pos

    r_layer, r_pos = layer_and_pos(lax.broadcasted_iota(jnp.int32, (n, n), 0))
    c_layer, c_pos = layer_and_pos(lax.broadcasted_iota(jnp.int32, (n, n), 1))
    same = r_layer == c_layer
    keep = same & ((r_pos < n_mem) | (r_pos >= c_pos))
    fill = jnp.where(same, -1e9, -jnp.inf).astype(F32)
    return keep, fill


def _loop(lo, hi, body):
    lax.fori_loop(lo, hi, lambda i, carry: (body(i), carry)[1], 0)


def _load_tiles(ref, lo, n, rows=slice(None)):
    return jnp.concatenate([ref[t, rows, :] for t in range(lo, lo + n)], axis=1)


def _store_operand(ref, lo, rows, val):
    for t in range(val.shape[1] // LANES):
        tile = val[:, t * LANES:(t + 1) * LANES].astype(BF16)
        ref[lo + t, rows, :] = tile.astype(ref.dtype)


def _kernel(x_hbm, mem0_ref, wq_hbm, wk_hbm, wv_hbm, wo_hbm, wg_hbm, wu_hbm, wd_hbm,
            out_hbm,
            wqkv, wo, wg, wu, wd, stage, xin, xs, xout, ha, ahead, h2, att2, h1, att1, hf, act,
            stage_sem, w_sem, x_sem, out_sem, *, n_mem, seg, n_seg):
    n_heads, dm_tiles = wqkv.shape[0] // 3, wqkv.shape[1]
    dh = LANES
    ff_tiles = wg.shape[0]
    scale = float(dh) ** -0.5
    n_groups = n_heads // HEAD_GROUP
    every = slice(None)
    mem_rows = slice(0, 2 * n_mem)
    first_rows = slice(2 * n_mem, 2 * n_mem + seg)
    second_rows = slice(2 * n_mem + seg, 2 * n_mem + 2 * seg)
    first_ahead = n_seg - AHEAD

    def rows(s):
        if isinstance(s, int):
            return slice(s * seg, (s + 1) * seg)
        return pl.ds(pl.multiple_of(s * seg, seg), seg)

    def attend(h_ref, att, n_layers, ahead_seg=None, fillers=()):
        keep, fill = _score_mask(n_layers, n_mem, seg)
        fillers = list(fillers)

        def operand(x):
            return x.astype(BF16).astype(h_ref.dtype)

        def project(g, which=(0, 1, 2)):
            if ahead_seg is None:
                h = _load_tiles(h_ref, 0, dm_tiles)
            else:
                h = jnp.concatenate([_load_tiles(h_ref, 0, dm_tiles, mem_rows),
                                     _load_tiles(h_ref, 0, dm_tiles, second_rows)], axis=0)
            out = []
            for i in which:
                tile = i * n_heads + g * HEAD_GROUP
                w = [pltpu.bitcast(wqkv[tile + j].reshape(dm_tiles * LANES // 2, dh), BF16)
                     for j in range(HEAD_GROUP)]
                y = _dot(h, jnp.concatenate(w, axis=1))
                heads = [y[:, j * dh:(j + 1) * dh] for j in range(HEAD_GROUP)]
                if ahead_seg is not None:
                    heads = [jnp.concatenate([z[mem_rows], ahead[tile + j, rows(ahead_seg), :],
                                              z[2 * n_mem:]], axis=0)
                             for j, z in enumerate(heads)]
                out.append([operand(z) for z in heads])
            return out

        def mix(g, probs, v):
            for i in range(HEAD_GROUP):
                att[g * HEAD_GROUP + i] = operand(_dot(probs[i], v[i]))

        q, k, v = project(0)
        pending = None
        for g in range(n_groups):
            probs = [operand(_softmax(jnp.where(keep, _dot_nt(q[i], k[i]) * scale, fill)))
                     for i in range(HEAD_GROUP)]
            if v is None:
                v, = project(g, (2,))
            if pending is not None:
                mix(*pending)
            pending = (g, probs, v)
            if g + 2 == n_groups and not fillers:
                (q, k), v = project(g + 1, (0, 1)), None
            elif g + 1 < n_groups:
                q, k, v = project(g + 1)
            elif fillers:
                fillers.pop(0)()
        mix(*pending)
        for f in fillers:
            f()

    def out_project(h_ref, att, segs, first_from_input):
        n_rows = len(segs) * n_mem
        a = _load_tiles(att, 0, n_heads)
        for j in range(0, dm_tiles, OUT_TILES):
            cols = slice(j * LANES, (j + OUT_TILES) * LANES)
            o = _dot(a, _load_tiles(wo, j, OUT_TILES))
            _store_operand(h_ref, j, slice(0, n_rows), o[0:n_rows])
            for l, s in enumerate(segs):
                if first_from_input and l == 0:
                    x = xin[rows(s), cols].astype(F32)
                else:
                    x = xs[rows(s), cols]
                xs[rows(s), cols] = x + o[n_rows + l * seg:n_rows + (l + 1) * seg]

    def ffn_norm(segs):
        for l, s in enumerate(segs):
            _store_operand(hf, 0, slice(l * seg, (l + 1) * seg), _layernorm(xs[rows(s), :]))

    def ffn_up(j):
        h = _load_tiles(hf, 0, dm_tiles)
        g = _dot(h, _load_tiles(wg, j, FF_TILES))
        u = _dot(h, _load_tiles(wu, j, FF_TILES))
        _store_operand(act, j, every, _gelu(g) * u)

    def ffn_down(segs):
        a = _load_tiles(act, 0, ff_tiles)
        for j in range(0, dm_tiles, OUT_TILES):
            cols = slice(j * LANES, (j + OUT_TILES) * LANES)
            o = _dot(a, _load_tiles(wd, j, OUT_TILES))
            for l, s in enumerate(segs):
                y = xs[rows(s), cols] + o[l * seg:(l + 1) * seg]
                xs[rows(s), cols] = y
                xout[rows(s), cols] = y.astype(BF16)

    def load_input(s):
        x = xin[rows(s), :].astype(F32)
        xs[rows(s), :] = x
        return _layernorm(x)

    chunk_rows = LANES * n_heads

    def stage_copy(src, c):
        return pltpu.make_async_copy(
            src.at[pl.ds(pl.multiple_of(c * chunk_rows, chunk_rows), chunk_rows), :],
            stage.at[c], stage_sem.at[c])

    def tile_copy(src, dst, t, sem):
        start = t * LANES if isinstance(t, int) else pl.multiple_of(t * LANES, LANES)
        return pltpu.make_async_copy(src.at[:, pl.ds(start, LANES)], dst.at[t], sem)

    def start_tiles(src, dst, sem):
        for t in range(dst.shape[0]):
            tile_copy(src, dst, t, sem).start()

    def wait_filled(buf, sem):
        pltpu.make_async_copy(buf, buf, sem).wait()

    def row_copy(src, dst, lo, hi, sem):
        return pltpu.make_async_copy(
            src.at[lo * seg:hi * seg, :], dst.at[lo * seg:hi * seg, :], sem)

    x_ahead = row_copy(x_hbm, xin, first_ahead, n_seg, x_sem.at[0])
    x_head = row_copy(x_hbm, xin, 0, LAG + 1, x_sem.at[1])
    x_rest = row_copy(x_hbm, xin, LAG + 1, first_ahead, x_sem.at[2])
    n_full = n_seg - LAG
    out_early = row_copy(xout, out_hbm, 0, n_full - 1, out_sem.at[0])
    out_mid = row_copy(xout, out_hbm, n_full - 1, n_seg - 2, out_sem.at[1])
    out_last = row_copy(xout, out_hbm, n_seg - 2, n_seg, out_sem.at[2])

    x_ahead.start()
    stage_copy(wq_hbm, 0).start()
    x_ahead.wait()
    for c in range(1, 3):
        stage_copy(wq_hbm, c).start()
    for s in range(AHEAD):
        x = xin[(first_ahead + s) * seg:(first_ahead + s + 1) * seg, :].astype(F32)
        _store_operand(ha, 0, slice(s * seg, (s + 1) * seg), _layernorm(x))

    pairs = n_heads // 2

    def retile(which, chunks):
        for c in chunks:
            wait_filled(stage.at[c], stage_sem.at[c])
        words = stage.bitcast(jnp.uint32)
        h = jnp.concatenate([ha[c] for c in chunks], axis=1)
        for g in range(n_groups):
            columns = []
            for j in range(g * HEAD_GROUP // 2, (g + 1) * HEAD_GROUP // 2):
                packed = [words[c, pl.ds(j, LANES, stride=pairs), :] for c in chunks]
                for half in range(2):
                    tile = which * n_heads + 2 * j + half
                    w = [pltpu.bitcast((p >> (16 * half)).astype(jnp.uint16), BF16)
                         for p in packed]
                    for c, wc in zip(chunks, w):
                        wqkv[tile, c] = pltpu.bitcast(wc, jnp.uint32)
                    columns.append(jnp.concatenate(w, axis=0))
            y = _dot(h, jnp.concatenate(columns, axis=1))
            for j in range(HEAD_GROUP):
                tile = which * n_heads + g * HEAD_GROUP + j
                old = jnp.where(chunks[0] == 0, 0.0, ahead[tile])
                ahead[tile] = old + y[:, j * dh:(j + 1) * dh]

    def stream_first(c):
        retile(0, [c])
        stage_copy(wk_hbm, c).start()

    def stream(n):
        which = n // n_iter
        chunks = [(n % n_iter) * STREAM_CHUNKS + j for j in range(STREAM_CHUNKS)]
        retile(which, chunks)
        for w, src in enumerate((wk_hbm, wv_hbm)):
            @pl.when(which == w)
            def _(src=src):
                for c in chunks:
                    stage_copy(src, c).start()

        @pl.when(which < 2)
        def _():
            tile_copy(wo_hbm, wo, n, w_sem.at[0]).start()

        pl.when(n == 2 * n_iter)(lambda: start_tiles(wg_hbm, wg, w_sem.at[1]))
        pl.when(n == 2 * n_iter + 2)(lambda: start_tiles(wu_hbm, wu, w_sem.at[2]))

    n_iter = dm_tiles // STREAM_CHUNKS
    assert 2 * n_iter == dm_tiles and n_iter > 2
    for c in range(3, dm_tiles):
        stage_copy(wq_hbm, c).start()
    x_head.start()
    _loop(0, STREAM_CHUNKS, stream_first)
    tile_copy(wo_hbm, wo, 0, w_sem.at[0]).start()
    _loop(1, 3 * n_iter, stream)
    start_tiles(wd_hbm, wd, w_sem.at[3])
    x_rest.start()

    x_head.wait()
    mem0 = mem0_ref[...].astype(F32)

    def ffn_only(segs):
        ffn_norm(segs)
        for j in ff_steps:
            ffn_up(j)
        ffn_down(segs)

    def single_step(s, next_tokens):
        attend(h1, att1, 1)
        _store_operand(h1, 0, slice(n_mem, n_mem + seg), next_tokens())
        out_project(h1, att1, (s,), False)

    def head_step(s):
        single_step(s, lambda: load_input(s + 1))

        @pl.when(s == LAG - 1)
        def _():
            for i, w in enumerate((wg, wu, wd)):
                wait_filled(w, w_sem.at[1 + i])
            x_rest.wait()
            ffn_only((0, 1))
            mem1 = _load_tiles(h1, 0, dm_tiles, slice(0, n_mem))
            _store_operand(h2, 0, mem_rows, jnp.concatenate([mem1, mem0], axis=0))
            _store_operand(h2, 0, first_rows, _layernorm(xin[rows(LAG), :].astype(F32)))
            _store_operand(h2, 0, second_rows, _layernorm(xs[rows(0), :]))

    def tail_step(k):
        s = n_full + k
        single_step(s, lambda: _layernorm(xs[rows(jnp.minimum(s + 1, n_seg - 1)), :]))

        @pl.when(k != 2)
        def _():
            ffn_only((jnp.where(k == 0, n_seg - 1, s - 1), jnp.where(k == 0, n_full - 1, s)))

        pl.when(k == 1)(out_mid.start)

    def full_step(t, projected_ahead):
        ff_segs = (t - 1, jnp.where(t == LAG, LAG - 2, t - LAG - 1))
        ffn_norm(ff_segs)
        attend(h2, att2, 2, t - first_ahead if projected_ahead else None,
               [functools.partial(ffn_up, j) for j in ff_steps])
        out_project(h2, att2, (t, t - LAG), True)
        if not projected_ahead:
            _store_operand(h2, 0, first_rows, _layernorm(xin[rows(t + 1), :].astype(F32)))
        _store_operand(h2, 0, second_rows, _layernorm(xs[rows(t + 1 - LAG), :]))
        ffn_down(ff_segs)

    ff_steps = range(0, ff_tiles, FF_TILES)
    _store_operand(h1, 0, slice(0, n_mem), mem0)
    _store_operand(h1, 0, slice(n_mem, n_mem + seg), load_input(0))

    wait_filled(wo, w_sem.at[0])
    _loop(0, LAG, head_step)
    _loop(LAG, first_ahead, lambda t: full_step(t, False))
    _loop(first_ahead, n_seg, lambda t: full_step(t, True))

    out_early.start()
    both = _load_tiles(h2, 0, dm_tiles, mem_rows).astype(F32)
    _store_operand(h1, 0, slice(0, n_mem), both[n_mem:])
    _store_operand(h1, 0, slice(n_mem, n_mem + seg),
                   _load_tiles(h2, 0, dm_tiles, second_rows).astype(F32))
    _loop(0, LAG, tail_step)

    out_last.start()
    out_early.wait()
    out_mid.wait()
    out_last.wait()


@functools.partial(jax.jit, static_argnames=("A_seg_len",))
def pallas_interleave_layers__memory_aug_recurrent_mem_tr__glu_gated_geglu__prompt_kernel(
    A_x: jax.Array,
    A_mem0: jax.Array,
    A_Wq: jax.Array,
    A_Wk: jax.Array,
    A_Wv: jax.Array,
    A_Wo: jax.Array,
    A_seg_len: int,
    B_x: jax.Array,
    B_w_gate: jax.Array,
    B_w_up: jax.Array,
    B_w_down: jax.Array,
):
    del B_x
    b, s, dm = A_x.shape
    _, n_heads, dh = A_Wq.shape
    n_mem = A_mem0.shape[1]
    dff = B_w_gate.shape[1]
    seg = int(A_seg_len)
    n_seg = s // seg
    assert b == 1 and dh == LANES and n_seg * seg == s and n_mem == 8 and seg % 16 == 0
    assert LAG == 4 and n_seg > 2 * LAG + AHEAD + 1
    hd = n_heads * dh
    full = 2 * (n_mem + seg)

    def tiled(n_rows, n_cols, dtype=BF16):
        return pltpu.VMEM((n_cols // LANES, n_rows, LANES), dtype)

    any_spec = pl.BlockSpec(memory_space=pl.ANY)
    out = pl.pallas_call(
        functools.partial(_kernel, n_mem=n_mem, seg=seg, n_seg=n_seg),
        out_shape=jax.ShapeDtypeStruct((s, dm), A_x.dtype),
        in_specs=[any_spec, pl.BlockSpec(memory_space=pltpu.VMEM)] + [any_spec] * 7,
        out_specs=any_spec,
        scratch_shapes=[
            pltpu.VMEM((3 * n_heads, dm // LANES, LANES // 2, dh), jnp.uint32),
            tiled(hd, dm),
            tiled(dm, dff), tiled(dm, dff), tiled(dff, dm),
            pltpu.VMEM((dm // LANES, LANES * n_heads, dh), BF16),
            pltpu.VMEM((s, dm), BF16),
            pltpu.VMEM((s, dm), F32),
            pltpu.VMEM((s, dm), BF16),
            tiled(AHEAD * seg, dm),
            tiled(AHEAD * seg, 3 * hd, F32),
            tiled(full, dm), tiled(full, hd),
            tiled(full // 2, dm, F32), tiled(full // 2, hd, F32),
            tiled(2 * seg, dm), tiled(2 * seg, dff),
            pltpu.SemaphoreType.DMA((dm // LANES,)),
            pltpu.SemaphoreType.DMA((4,)),
            pltpu.SemaphoreType.DMA((3,)),
            pltpu.SemaphoreType.DMA((3,)),
        ],
        compiler_params=pltpu.CompilerParams(vmem_limit_bytes=110 * 1024 * 1024),
    )(
        A_x.reshape(s, dm),
        A_mem0.reshape(n_mem, dm),
        A_Wq.reshape(dm * n_heads, dh),
        A_Wk.reshape(dm * n_heads, dh),
        A_Wv.reshape(dm * n_heads, dh),
        A_Wo.reshape(hd, dm),
        B_w_gate,
        B_w_up,
        B_w_down,
    )
    return out.reshape(b, s, dm)
```
